```python
import jax
import jax.numpy as jnp

def _softmax(x, axis=-1):
    return jax.nn.softmax(x, axis=axis)
def _gelu(x):
    return jax.nn.gelu(x, approximate=True)
def _silu(x):
    return jax.nn.silu(x)
def _sigmoid(x):
    return jax.nn.sigmoid(x)
def _layernorm(x, axis=-1, eps=1e-5):
    m = jnp.mean(x, axis=axis, keepdims=True)
    v = jnp.var(x, axis=axis, keepdims=True)
    return (x - m) / jnp.sqrt(v + eps)
def _scatter_add(tgt, idx, src, axis=0):
    return tgt.at[idx].add(src)
def _segment_sum(src, seg, n):
    return jax.ops.segment_sum(src, seg, n)
class _Rng:
    def __init__(self, key):
        self._k = key
    def _next(self):
        self._k, sub = jax.random.split(self._k)
        return sub
    def normal(self, shape):
        return jax.random.normal(self._next(), shape, dtype=jnp.bfloat16)
    def randint(self, lo, hi, shape):
        return jax.random.randint(self._next(), shape, lo, hi, dtype=jnp.int32)
    def uniform(self, shape, lo=0.0, hi=1.0):
        return jax.random.uniform(self._next(), shape, jnp.bfloat16, lo, hi)
    def permutation(self, n):
        return jax.random.permutation(self._next(), n)


kernel_name = 'parallel_sum__gqa_block_cached__moe_arch_mod__decode'

def setup_inputs():
    _rng = _Rng(jax.random.key(int.from_bytes(__import__("os").urandom(4), "little")))
    _w = (lambda a: (lambda t: t.astype(jnp.bfloat16) if jnp.issubdtype(t.dtype, jnp.floating) else t)(jnp.asarray(a)))
    def _A_setup():
        B, Sq, D = 1, 1, 448
        Hq, Hkv, Sk, Dh = 16, 8, 65536, 256
        assert Hq % Hkv == 0, (Hq, Hkv)
        return {
            "x": _w((lambda *s: _rng.normal(s) * 0.05)(B, Sq, D)),
            "k_cache": _w((lambda *s: _rng.normal(s) * 0.05)(B, Hkv, Sk, Dh)),
            "v_cache": _w((lambda *s: _rng.normal(s) * 0.05)(B, Hkv, Sk, Dh)),
            "wq": _w((lambda *s: _rng.normal(s) * 0.05)(D, Hq * Dh) * (D ** -0.5)),
            "wo": _w((lambda *s: _rng.normal(s) * 0.05)(Hq * Dh, D) * ((Hq * Dh) ** -0.5)),
        }
    _A_in = _A_setup()

    def _B_setup():
        B, S, D, F, C = 1, 1, 448, 1792, 1
        return {
            "x": _w((lambda *s: _rng.normal(s) * 0.05)(B, S, D)),
            "w_r": _w((lambda *s: _rng.normal(s) * 0.05)(D)),
            "w_gate": _w((lambda *s: _rng.normal(s) * 0.05)(D, F)),
            "w_up": _w((lambda *s: _rng.normal(s) * 0.05)(D, F)),
            "w_down": _w((lambda *s: _rng.normal(s) * 0.05)(F, D)),
        }
    _B_in = _B_setup()

    return {
        "A_x": _A_in["x"],
        "A_k_cache": _A_in["k_cache"],
        "A_v_cache": _A_in["v_cache"],
        "A_wq": _A_in["wq"],
        "A_wo": _A_in["wo"],
        "B_x": _B_in["x"],
        "B_w_r": _B_in["w_r"],
        "B_w_gate": _B_in["w_gate"],
        "B_w_up": _B_in["w_up"],
        "B_w_down": _B_in["w_down"],
    }

def reference(A_x, A_k_cache, A_v_cache, A_wq, A_wo, B_x, B_w_r, B_w_gate, B_w_up, B_w_down):
    def _A_ref(x, k_cache, v_cache, wq, wo):
        B, Sq, D = x.shape
        Hq, Dh = 16, 256
        Hkv = k_cache.shape[1]
        rep = Hq // Hkv
        q = (lambda x, *d: x.transpose(*d))((x @ wq).reshape(B, Sq, Hq, Dh), 0, 2, 1, 3)
        k = jnp.repeat(k_cache, rep, axis=1)
        v = jnp.repeat(v_cache, rep, axis=1)
        scores = jnp.einsum("bhqd,bhkd->bhqk", q, k) * (Dh ** -0.5)
        p = _softmax(scores, axis=-1)
        o = jnp.einsum("bhqk,bhkd->bhqd", p, v)
        return (lambda x, *d: x.transpose(*d))(o, 0, 2, 1, 3).reshape(B, Sq, Hq * Dh) @ wo

    def _B_ref(x, w_r, w_gate, w_up, w_down):
        B, S, D = x.shape
        C = 1
        r = x @ w_r
        idx = jnp.argsort(-r, axis=-1)[:, :C]
        idx_e = jnp.repeat(idx.reshape(B, C, 1), D, axis=2)
        x_sel = jnp.take_along_axis(x, idx_e, axis=1)
        g = _silu(x_sel @ w_gate)
        u = x_sel @ w_up
        y = (g * u) @ w_down
        r_sel = _sigmoid(jnp.take_along_axis(r, idx, axis=1))
        y = y * r_sel.reshape(B, C, 1)
        b_off = (jnp.arange(B) * S).reshape(B, 1)
        flat_idx = (idx + b_off).reshape(B * C)
        zero = (x * 0.0).reshape(B * S, D)
        upd = _scatter_add(zero, flat_idx, y.reshape(B * C, D), axis=0)
        return x + upd.reshape(B, S, D)

    x = A_x
    xn = _layernorm(x, axis=-1)
    return x + _A_ref(xn, A_k_cache, A_v_cache, A_wq, A_wo) + _B_ref(xn, B_w_r, B_w_gate, B_w_up, B_w_down)
```

```python
import functools

import jax
import jax.numpy as jnp
import jax.experimental.pallas as pl
import jax.experimental.pallas.tpu as pltpu


HI = 0
LO = 1

U = 512
PIECES = (112, 112, 112, 112, 64)
AK = 3
AV = 6
CB = 256
NEG = -1e30


def _kernel(x_hbm, k_hbm, v_hbm, wq_hbm, wot_hbm, wr_hbm, wg_hbm, wu_hbm, wdt_hbm,
            o_hbm,
            xbuf, wrbuf, obuf, kbuf, vbuf, wqbuf, wobuf, wgbuf, wubuf, wdbuf,
            xn_scr, q_scr, out_scr,
            ksem, vsem, wqsem, wosem, msem,
            *, n_kv, sk, dh, d_model, rep):
    ns = len(PIECES)
    starts = [sum(PIECES[:j]) for j in range(ns)]
    nb = U // CB
    upb = sk // U
    n_units = n_kv * upb
    nk = AK + 1
    nv = AV + 1
    hw = rep * dh
    f32 = jnp.float32
    bf16 = jnp.bfloat16

    def k_copy(u, j):
        slot = u % nk
        return pltpu.make_async_copy(
            k_hbm.at[pl.ds(u * U + starts[j], PIECES[j])],
            kbuf.at[slot, pl.ds(starts[j], PIECES[j])], ksem.at[slot])

    def k_wait(u):
        slot = u % nk
        pltpu.make_async_copy(kbuf.at[slot], kbuf.at[slot], ksem.at[slot]).wait()

    def v_copy(u, j):
        slot = u % nv
        return pltpu.make_async_copy(
            v_hbm.at[pl.ds(u * U + starts[j], PIECES[j])],
            vbuf.at[slot, pl.ds(starts[j], PIECES[j])], vsem.at[slot, j])

    def wq_copy(h):
        col = pl.multiple_of(h * hw, hw)
        return pltpu.make_async_copy(wq_hbm.at[:, pl.ds(col, hw)], wqbuf.at[h], wqsem.at[h])

    def wo_copy(h):
        col = pl.multiple_of(h * hw, hw)
        return pltpu.make_async_copy(wot_hbm.at[:, pl.ds(col, hw)], wobuf.at[h], wosem.at[h])

    x_copy = pltpu.make_async_copy(x_hbm, xbuf, msem.at[0])
    wr_copy = pltpu.make_async_copy(wr_hbm, wrbuf, msem.at[1])
    wg_copy = pltpu.make_async_copy(wg_hbm, wgbuf, msem.at[2])
    wu_copy = pltpu.make_async_copy(wu_hbm, wubuf, msem.at[3])
    wd_copy = pltpu.make_async_copy(wdt_hbm, wdbuf, msem.at[4])
    out_copy = pltpu.make_async_copy(obuf, o_hbm, msem.at[5])

    x_copy.start(priority=HI)
    wr_copy.start(priority=HI)
    wq_copy(0).start(priority=HI)
    for u in range(AK + 1):
        for j in range(ns):
            k_copy(u, j).start(priority=HI)
    for u in range(AV):
        for j in range(ns):
            v_copy(u, j).start(priority=LO)

    x_copy.wait()
    x = xbuf[0].astype(f32)
    mu = jnp.mean(x, axis=1, keepdims=True)
    xc = x - mu
    var = jnp.mean(xc * xc, axis=1, keepdims=True)
    xn = (xc / jnp.sqrt(var + 1e-5)).astype(bf16)
    xn_scr[...] = jnp.broadcast_to(xn, (8, d_model))

    row = jax.lax.broadcasted_iota(jnp.int32, (8, dh), 0)
    top = row < 4

    def make_q(h):
        qf = jnp.dot(xn_scr[...], wqbuf[h], preferred_element_type=f32)
        qh = jnp.where(top, qf[:, :dh], qf[:, dh:]).astype(bf16)
        q_scr[h] = (qh.astype(f32) * (dh ** -0.5)).astype(bf16)

    wq_copy(0).wait()
    make_q(0)
    out_scr[...] = jnp.zeros(out_scr.shape, f32)

    def qk(u, b):
        kk = kbuf[u % nk, pl.ds(b * CB, CB), :]
        return jax.lax.dot_general(q_scr[u // upb], kk, (((1,), (1,)), ((), ())),
                                   preferred_element_type=f32)

    def softmax(u, s_parts, m, l):
        first = (u % upb) == 0
        m_prev = jnp.where(first, NEG, m)
        l_prev = jnp.where(first, 0.0, l)
        s = jnp.concatenate(s_parts, axis=1)
        m_new = jnp.maximum(m_prev, jnp.max(s, axis=1, keepdims=True))
        p = jnp.exp(s - m_new)
        alpha = jnp.exp(m_prev - m_new)
        ps = p[:, 0:128]
        for c in range(1, U // 128):
            ps = ps + p[:, c * 128:(c + 1) * 128]
        return p.astype(bf16), alpha, m_new, alpha * l_prev + ps

    def pv(u, p, b):
        vv = vbuf[u % nv, pl.ds(b * CB, CB), :]
        return jnp.dot(p[:, b * CB:(b + 1) * CB], vv, preferred_element_type=f32)

    k_wait(0)
    s0 = [qk(0, b) for b in range(nb)]
    p0, a0, m0, l0 = softmax(0, s0, jnp.full((8, 1), NEG, f32), jnp.zeros((8, 128), f32))
    acc0 = jnp.zeros((8, dh), f32)

    plan = [[("qk", 0)], [("qk", 1)], [("sm",)], [("pv", 0)], [("pv", 1)]]

    def body(u, carry, issue_k, issue_v, has_next):
        p, alpha, m, l, acc = carry
        h = u // upb
        r = u % upb
        s_parts = [None] * nb
        pv_sum = None
        nxt = (p, alpha, m, l)
        for j in range(ns):
            v_copy(u, j).wait()
            if issue_k:
                k_copy(u + 1 + AK, j).start(priority=HI)
            if issue_v:
                v_copy(u + AV, j).start(priority=LO)
            for item in plan[j]:
                if item[0] == "qk":
                    if has_next:
                        if item[1] == 0:
                            k_wait(u + 1)
                        s_parts[item[1]] = qk(u + 1, item[1])
                elif item[0] == "sm":
                    if has_next:
                        nxt = softmax(u + 1, s_parts, m, l)
                else:
                    res = pv(u, p, item[1])
                    pv_sum = res if pv_sum is None else pv_sum + res
        acc = alpha * acc + pv_sum

        @pl.when(r == 0)
        def _():
            @pl.when(h < n_kv - 1)
            def _():
                wq_copy(h + 1).start(priority=LO)
            wo_copy(h).start(priority=LO)

            @pl.when(h == 0)
            def _():
                wg_copy.start(priority=LO)

            @pl.when(h == 1)
            def _():
                wu_copy.start(priority=LO)

            @pl.when(h == 2)
            def _():
                wd_copy.start(priority=LO)

        @pl.when(jnp.logical_and(r == upb // 2, h < n_kv - 1))
        def _():
            wq_copy(h + 1).wait()
            make_q(h + 1)

        @pl.when(jnp.logical_and(r == upb // 4, h == 4))
        def _():
            wg_copy.wait()
            wu_copy.wait()
            wd_copy.wait()
            wr_copy.wait()
            xb = xn_scr[...]
            g = jnp.dot(xb, wgbuf[...], preferred_element_type=f32).astype(bf16).astype(f32)
            up = jnp.dot(xb, wubuf[...], preferred_element_type=f32).astype(bf16).astype(f32)
            g = (g * jax.nn.sigmoid(g)).astype(bf16)
            hid = (g.astype(f32) * up).astype(bf16)
            y = jax.lax.dot_general(hid, wdbuf[...], (((1,), (1,)), ((), ())),
                                    preferred_element_type=f32)
            xf = xb.astype(f32)
            wr = wrbuf[...].astype(f32).reshape(1, d_model)
            rs = jax.nn.sigmoid(jnp.sum(xf * wr, axis=1, keepdims=True))
            rows = jax.lax.broadcasted_iota(jnp.int32, (8, d_model), 0)
            base = xf + xf * 0.0 + y * rs
            out_scr[...] += jnp.where(rows == 0, base, 0.0)

        @pl.when(r == upb - 1)
        def _():
            o = acc / jnp.sum(l, axis=1, keepdims=True)
            sel0 = row == 0
            sel1 = row == 4
            lhs = jnp.concatenate([jnp.where(sel0, o, 0.0), jnp.where(sel1, o, 0.0)],
                                  axis=1).astype(bf16)
            wo_copy(h).wait()
            out_scr[...] += jax.lax.dot_general(lhs, wobuf[h], (((1,), (1,)), ((), ())),
                                                preferred_element_type=f32)
        return nxt + (acc,)

    carry = (p0, a0, m0, l0, acc0)
    n1 = n_units - max(AV, AK + 1)
    carry = jax.lax.fori_loop(0, n1, lambda u, c: body(u, c, True, True, True), carry)
    if AV > AK + 1:
        carry = jax.lax.fori_loop(n1, n_units - AK - 1,
                                  lambda u, c: body(u, c, True, False, True), carry)
    elif AK + 1 > AV:
        carry = jax.lax.fori_loop(n1, n_units - AV,
                                  lambda u, c: body(u, c, False, True, True), carry)
    n2 = n_units - min(AV, AK + 1)
    carry = jax.lax.fori_loop(n2, n_units - 1,
                              lambda u, c: body(u, c, False, False, True), carry)
    body(n_units - 1, carry, False, False, False)

    res = jnp.sum(out_scr[...], axis=0, keepdims=True) + xbuf[0].astype(f32)
    obuf[0] = res.astype(obuf.dtype)
    out_copy.start()
    out_copy.wait()


@jax.jit
def pallas_parallel_sum__gqa_block_cached__moe_arch_mod__decode_kernel(
    A_x: jax.Array,
    A_k_cache: jax.Array,
    A_v_cache: jax.Array,
    A_wq: jax.Array,
    A_wo: jax.Array,
    B_x: jax.Array,
    B_w_r: jax.Array,
    B_w_gate: jax.Array,
    B_w_up: jax.Array,
    B_w_down: jax.Array,
):
    del B_x
    _, n_kv, sk, dh = A_k_cache.shape
    d_model = A_x.shape[-1]
    hq = A_wq.shape[1] // dh
    rep = hq // n_kv
    assert rep == 2 and A_x.shape == (1, 1, d_model)
    ffn = B_w_gate.shape[1]
    hw = rep * dh
    ns = len(PIECES)
    bf16 = jnp.bfloat16

    k2 = A_k_cache.reshape(n_kv * sk, dh)
    v2 = A_v_cache.reshape(n_kv * sk, dh)
    wot = A_wo.T
    wdt = B_w_down.T

    kernel = functools.partial(_kernel, n_kv=n_kv, sk=sk, dh=dh, d_model=d_model, rep=rep)
    return pl.pallas_call(
        kernel,
        out_shape=jax.ShapeDtypeStruct((1, 1, d_model), A_x.dtype),
        in_specs=[pl.BlockSpec(memory_space=pl.ANY)] * 9,
        out_specs=pl.BlockSpec(memory_space=pl.ANY),
        scratch_shapes=[
            pltpu.VMEM((1, 1, d_model), bf16),
            pltpu.VMEM((d_model,), bf16),
            pltpu.VMEM((1, 1, d_model), bf16),
            pltpu.VMEM((AK + 1, U, dh), bf16),
            pltpu.VMEM((AV + 1, U, dh), bf16),
            pltpu.VMEM((n_kv, d_model, hw), bf16),
            pltpu.VMEM((n_kv, d_model, hw), bf16),
            pltpu.VMEM((d_model, ffn), bf16),
            pltpu.VMEM((d_model, ffn), bf16),
            pltpu.VMEM((d_model, ffn), bf16),
            pltpu.VMEM((8, d_model), bf16),
            pltpu.VMEM((n_kv, 8, dh), bf16),
            pltpu.VMEM((8, d_model), jnp.float32),
            pltpu.SemaphoreType.DMA((AK + 1,)),
            pltpu.SemaphoreType.DMA((AV + 1, ns)),
            pltpu.SemaphoreType.DMA((n_kv,)),
            pltpu.SemaphoreType.DMA((n_kv,)),
            pltpu.SemaphoreType.DMA((6,)),
        ],
        compiler_params=pltpu.CompilerParams(vmem_limit_bytes=64 * 1024 * 1024),
    )(A_x, k2, v2, A_wq, wot, B_w_r, B_w_gate, B_w_up, wdt)
```

```python
import functools

import jax
import jax.numpy as jnp
import jax.experimental.pallas as pl
import jax.experimental.pallas.tpu as pltpu


HI = 0
LO = 1

U = 512
KP = (72, 104, 40, 96, 104, 96)
VP = (48, 112, 48, 96, 120, 88)
PLAN = [[('qk', 0), ('qk', 1)], [('sm',)], [], [], [], [('pv', 0), ('pv', 1)]]
AK = 4
AV = 6
CB = 256
NEG = -1e30
NO_BOUNDS = True


def _auto_plan(vp, nb):
    ns = len(vp)
    plan = [[] for _ in range(ns)]
    ends = [sum(vp[:j + 1]) for j in range(ns)]
    pv_seg = [min(j for j in range(ns) if ends[j] >= (b + 1) * CB) for b in range(nb)]
    free = [j for j in range(ns)]
    items = [("qk", b) for b in range(nb)] + [("sm",)]
    seg = ns - 1
    pv_at = {}
    for b in reversed(range(nb)):
        pv_at[b] = max(seg, pv_seg[b])
        seg -= 1
        if seg < pv_seg[max(b - 1, 0)]:
            seg = pv_seg[max(b - 1, 0)]
    used = set(pv_at.values())
    rest = [j for j in range(ns) if j not in used]
    for i, it in enumerate(items):
        j = rest[i] if i < len(rest) else rest[-1] if rest else 0
        plan[j].append(it)
    for b in range(nb):
        plan[pv_at[b]].append(("pv", b))
    return plan


def _kernel(x_hbm, k_hbm, v_hbm, wq_hbm, wot_hbm, wr_hbm, wg_hbm, wu_hbm, wdt_hbm,
            o_hbm,
            xbuf, wrbuf, obuf, kbuf, vbuf, wqbuf, wobuf, wgbuf, wubuf, wdbuf,
            xn_scr, q_scr, out_scr,
            ksem, vsem, wqsem, wosem, msem,
            *, n_kv, sk, dh, d_model, rep):
    ns = len(VP)
    assert len(KP) == ns and sum(KP) == U and sum(VP) == U
    kstarts = [sum(KP[:j]) for j in range(ns)]
    vstarts = [sum(VP[:j]) for j in range(ns)]
    nb = U // CB
    upb = sk // U
    n_units = n_kv * upb
    nk = AK + 1
    nv = AV + 1
    hw = rep * dh
    f32 = jnp.float32
    bf16 = jnp.bfloat16

    def k_copy(u, j):
        slot = u % nk
        return pltpu.make_async_copy(
            k_hbm.at[pl.ds(u * U + kstarts[j], KP[j])],
            kbuf.at[slot, pl.ds(kstarts[j], KP[j])], ksem.at[slot])

    def k_wait(u):
        slot = u % nk
        pltpu.make_async_copy(kbuf.at[slot], kbuf.at[slot], ksem.at[slot]).wait()

    def v_copy(u, j):
        slot = u % nv
        return pltpu.make_async_copy(
            v_hbm.at[pl.ds(u * U + vstarts[j], VP[j])],
            vbuf.at[slot, pl.ds(vstarts[j], VP[j])], vsem.at[slot, j])

    def wq_copy(h):
        col = pl.multiple_of(h * hw, hw)
        return pltpu.make_async_copy(wq_hbm.at[:, pl.ds(col, hw)], wqbuf.at[h], wqsem.at[h])

    def wo_copy(h):
        col = pl.multiple_of(h * hw, hw)
        return pltpu.make_async_copy(wot_hbm.at[:, pl.ds(col, hw)], wobuf.at[h], wosem.at[h])

    x_copy = pltpu.make_async_copy(x_hbm, xbuf, msem.at[0])
    wr_copy = pltpu.make_async_copy(wr_hbm, wrbuf, msem.at[1])
    wg_copy = pltpu.make_async_copy(wg_hbm, wgbuf, msem.at[2])
    wu_copy = pltpu.make_async_copy(wu_hbm, wubuf, msem.at[3])
    wd_copy = pltpu.make_async_copy(wdt_hbm, wdbuf, msem.at[4])
    out_copy = pltpu.make_async_copy(obuf, o_hbm, msem.at[5])

    x_copy.start(priority=HI)
    wr_copy.start(priority=HI)
    wq_copy(0).start(priority=HI)
    for u in range(AK + 1):
        for j in range(ns):
            k_copy(u, j).start(priority=HI)
    for u in range(AV):
        for j in range(ns):
            v_copy(u, j).start(priority=LO)

    x_copy.wait()
    x = xbuf[0].astype(f32)
    mu = jnp.mean(x, axis=1, keepdims=True)
    xc = x - mu
    var = jnp.mean(xc * xc, axis=1, keepdims=True)
    xn = (xc / jnp.sqrt(var + 1e-5)).astype(bf16)
    xn_scr[...] = jnp.broadcast_to(xn, (8, d_model))

    row = jax.lax.broadcasted_iota(jnp.int32, (8, dh), 0)
    top = row < 4

    def make_q(h):
        qf = jnp.dot(xn_scr[...], wqbuf[h], preferred_element_type=f32)
        qh = jnp.where(top, qf[:, :dh], qf[:, dh:]).astype(bf16)
        q_scr[h] = (qh.astype(f32) * (dh ** -0.5)).astype(bf16)

    wq_copy(0).wait()
    make_q(0)
    out_scr[...] = jnp.zeros(out_scr.shape, f32)

    def qk(u, b):
        kk = kbuf[u % nk, pl.ds(b * CB, CB), :]
        return jax.lax.dot_general(q_scr[u // upb], kk, (((1,), (1,)), ((), ())),
                                   preferred_element_type=f32)

    def softmax(u, s_parts, m, l):
        first = (u % upb) == 0
        m_prev = jnp.where(first, NEG, m)
        l_prev = jnp.where(first, 0.0, l)
        s = jnp.concatenate(s_parts, axis=1)
        m_new = jnp.maximum(m_prev, jnp.max(s, axis=1, keepdims=True))
        p = jnp.exp(s - m_new)
        alpha = jnp.exp(m_prev - m_new)
        ps = p[:, 0:128]
        for c in range(1, U // 128):
            ps = ps + p[:, c * 128:(c + 1) * 128]
        return p.astype(bf16), alpha, m_new, alpha * l_prev + ps

    def pv(u, p, b):
        vv = vbuf[u % nv, pl.ds(b * CB, CB), :]
        return jnp.dot(p[:, b * CB:(b + 1) * CB], vv, preferred_element_type=f32)

    k_wait(0)
    s0 = [qk(0, b) for b in range(nb)]
    p0, a0, m0, l0 = softmax(0, s0, jnp.full((8, 1), NEG, f32), jnp.zeros((8, 128), f32))
    acc0 = jnp.zeros((8, dh), f32)

    plan = PLAN if PLAN is not None else _auto_plan(VP, nb)

    def body(u, carry, issue_k, issue_v, has_next):
        p, alpha, m, l, acc = carry
        h = u // upb
        r = u % upb
        s_parts = [None] * nb
        pv_sum = None
        nxt = (p, alpha, m, l)
        for j in range(ns):
            v_copy(u, j).wait()
            if issue_k:
                k_copy(u + 1 + AK, j).start(priority=HI)
            if issue_v:
                v_copy(u + AV, j).start(priority=LO)
            for item in plan[j]:
                if item[0] == "qk":
                    if has_next:
                        if item[1] == 0:
                            k_wait(u + 1)
                        s_parts[item[1]] = qk(u + 1, item[1])
                elif item[0] == "sm":
                    if has_next:
                        nxt = softmax(u + 1, s_parts, m, l)
                else:
                    res = pv(u, p, item[1])
                    pv_sum = res if pv_sum is None else pv_sum + res
        acc = alpha * acc + pv_sum

        @pl.when(r == 0)
        def _():
            @pl.when(h < n_kv - 1)
            def _():
                wq_copy(h + 1).start(priority=LO)
            wo_copy(h).start(priority=LO)

            @pl.when(h == 0)
            def _():
                wg_copy.start(priority=LO)

            @pl.when(h == 1)
            def _():
                wu_copy.start(priority=LO)

            @pl.when(h == 2)
            def _():
                wd_copy.start(priority=LO)

        @pl.when(jnp.logical_and(r == upb // 2, h < n_kv - 1))
        def _():
            wq_copy(h + 1).wait()
            make_q(h + 1)

        @pl.when(jnp.logical_and(r == upb // 4, h == 4))
        def _():
            wg_copy.wait()
            wu_copy.wait()
            wd_copy.wait()
            wr_copy.wait()
            xb = xn_scr[...]
            g = jnp.dot(xb, wgbuf[...], preferred_element_type=f32).astype(bf16).astype(f32)
            up = jnp.dot(xb, wubuf[...], preferred_element_type=f32).astype(bf16).astype(f32)
            g = (g * jax.nn.sigmoid(g)).astype(bf16)
            hid = (g.astype(f32) * up).astype(bf16)
            y = jax.lax.dot_general(hid, wdbuf[...], (((1,), (1,)), ((), ())),
                                    preferred_element_type=f32)
            xf = xb.astype(f32)
            wr = wrbuf[...].astype(f32).reshape(1, d_model)
            rs = jax.nn.sigmoid(jnp.sum(xf * wr, axis=1, keepdims=True))
            rows = jax.lax.broadcasted_iota(jnp.int32, (8, d_model), 0)
            base = xf + xf * 0.0 + y * rs
            out_scr[...] += jnp.where(rows == 0, base, 0.0)

        @pl.when(r == upb - 1)
        def _():
            o = acc / jnp.sum(l, axis=1, keepdims=True)
            sel0 = row == 0
            sel1 = row == 4
            lhs = jnp.concatenate([jnp.where(sel0, o, 0.0), jnp.where(sel1, o, 0.0)],
                                  axis=1).astype(bf16)
            wo_copy(h).wait()
            out_scr[...] += jax.lax.dot_general(lhs, wobuf[h], (((1,), (1,)), ((), ())),
                                                preferred_element_type=f32)
        return nxt + (acc,)

    carry = (p0, a0, m0, l0, acc0)
    n1 = n_units - max(AV, AK + 1)
    carry = jax.lax.fori_loop(0, n1, lambda u, c: body(u, c, True, True, True), carry)
    if AV > AK + 1:
        carry = jax.lax.fori_loop(n1, n_units - AK - 1,
                                  lambda u, c: body(u, c, True, False, True), carry)
    elif AK + 1 > AV:
        carry = jax.lax.fori_loop(n1, n_units - AV,
                                  lambda u, c: body(u, c, False, True, True), carry)
    n2 = n_units - min(AV, AK + 1)
    carry = jax.lax.fori_loop(n2, n_units - 1,
                              lambda u, c: body(u, c, False, False, True), carry)
    body(n_units - 1, carry, False, False, False)

    res = jnp.sum(out_scr[...], axis=0, keepdims=True) + xbuf[0].astype(f32)
    obuf[0] = res.astype(obuf.dtype)
    out_copy.start()
    out_copy.wait()


@jax.jit
def pallas_parallel_sum__gqa_block_cached__moe_arch_mod__decode_kernel(
    A_x: jax.Array,
    A_k_cache: jax.Array,
    A_v_cache: jax.Array,
    A_wq: jax.Array,
    A_wo: jax.Array,
    B_x: jax.Array,
    B_w_r: jax.Array,
    B_w_gate: jax.Array,
    B_w_up: jax.Array,
    B_w_down: jax.Array,
):
    del B_x
    _, n_kv, sk, dh = A_k_cache.shape
    d_model = A_x.shape[-1]
    hq = A_wq.shape[1] // dh
    rep = hq // n_kv
    assert rep == 2 and A_x.shape == (1, 1, d_model)
    ffn = B_w_gate.shape[1]
    hw = rep * dh
    ns = len(VP)
    bf16 = jnp.bfloat16

    k2 = A_k_cache.reshape(n_kv * sk, dh)
    v2 = A_v_cache.reshape(n_kv * sk, dh)
    wot = A_wo.T
    wdt = B_w_down.T

    kernel = functools.partial(_kernel, n_kv=n_kv, sk=sk, dh=dh, d_model=d_model, rep=rep)
    return pl.pallas_call(
        kernel,
        out_shape=jax.ShapeDtypeStruct((1, 1, d_model), A_x.dtype),
        in_specs=[pl.BlockSpec(memory_space=pl.ANY)] * 9,
        out_specs=pl.BlockSpec(memory_space=pl.ANY),
        scratch_shapes=[
            pltpu.VMEM((1, 1, d_model), bf16),
            pltpu.VMEM((d_model,), bf16),
            pltpu.VMEM((1, 1, d_model), bf16),
            pltpu.VMEM((AK + 1, U, dh), bf16),
            pltpu.VMEM((AV + 1, U, dh), bf16),
            pltpu.VMEM((n_kv, d_model, hw), bf16),
            pltpu.VMEM((n_kv, d_model, hw), bf16),
            pltpu.VMEM((d_model, ffn), bf16),
            pltpu.VMEM((d_model, ffn), bf16),
            pltpu.VMEM((d_model, ffn), bf16),
            pltpu.VMEM((8, d_model), bf16),
            pltpu.VMEM((n_kv, 8, dh), bf16),
            pltpu.VMEM((8, d_model), jnp.float32),
            pltpu.SemaphoreType.DMA((AK + 1,)),
            pltpu.SemaphoreType.DMA((AV + 1, ns)),
            pltpu.SemaphoreType.DMA((n_kv,)),
            pltpu.SemaphoreType.DMA((n_kv,)),
            pltpu.SemaphoreType.DMA((6,)),
        ],
        compiler_params=pltpu.CompilerParams(vmem_limit_bytes=64 * 1024 * 1024,
                                             disable_bounds_checks=NO_BOUNDS),
    )(A_x, k2, v2, A_wq, wot, B_w_r, B_w_gate, B_w_up, wdt)
```

```python
import functools

import jax
import jax.numpy as jnp
import jax.experimental.pallas as pl
import jax.experimental.pallas.tpu as pltpu


HI = 0
LO = 1

U = 512
KP = (56, 128, 24, 104, 120, 80)
VP = (48, 120, 48, 80, 128, 88)
PLAN = [[('qk', 0), ('qk', 1)], [('sm',)], [], [], [], [('pv', 0), ('pv', 1)]]
AK = 4
AV = 6
CB = 256
NEG = -1e30
NO_BOUNDS = True
SPREAD = True
XEV = 1
XPRIO = 0
KEV = None
VFIRST = False
PADK = 0
PADV = 0
OFFK = 0
OFFV = 0
G = 1


def _auto_plan(vp, nb):
    ns = len(vp)
    plan = [[] for _ in range(ns)]
    ends = [sum(vp[:j + 1]) for j in range(ns)]
    pv_seg = [min(j for j in range(ns) if ends[j] >= (b + 1) * CB) for b in range(nb)]
    free = [j for j in range(ns)]
    items = [("qk", b) for b in range(nb)] + [("sm",)]
    seg = ns - 1
    pv_at = {}
    for b in reversed(range(nb)):
        pv_at[b] = max(seg, pv_seg[b])
        seg -= 1
        if seg < pv_seg[max(b - 1, 0)]:
            seg = pv_seg[max(b - 1, 0)]
    used = set(pv_at.values())
    rest = [j for j in range(ns) if j not in used]
    for i, it in enumerate(items):
        j = rest[i] if i < len(rest) else rest[-1] if rest else 0
        plan[j].append(it)
    for b in range(nb):
        plan[pv_at[b]].append(("pv", b))
    return plan


def _kernel(x_hbm, k_hbm, v_hbm, wq_hbm, wot_hbm, wr_hbm, wg_hbm, wu_hbm, wdt_hbm,
            o_hbm,
            xbuf, wrbuf, obuf, padk, kbuf, padv, vbuf, wqbuf, wobuf, wgbuf, wubuf, wdbuf,
            xn_scr, q_scr, out_scr,
            ksem, vsem, wqsem, wosem, msem,
            *, n_kv, sk, dh, d_model, rep):
    ns = len(VP)
    nkp = len(KP)
    kev = list(KEV) if KEV is not None else list(range(nkp))
    assert len(kev) == nkp and max(kev) < ns and sum(KP) == U and sum(VP) == U
    kstarts = [sum(KP[:j]) for j in range(nkp)]
    vstarts = [sum(VP[:j]) for j in range(ns)]
    nb = U // CB
    upb = sk // U
    n_units = n_kv * upb
    nk = AK + 1
    nv = AV + 1
    hw = rep * dh
    f32 = jnp.float32
    bf16 = jnp.bfloat16

    gs = U // G
    for st, sz in list(zip(kstarts, KP)) + list(zip(vstarts, VP)):
        assert st // gs == (st + sz - 1) // gs

    def hbm_row(u, start):
        if G == 1:
            return u * U + start
        return (u // upb) * sk + (start // gs) * (sk // G) + (u % upb) * gs + start % gs

    def dbg(row, off, size):
        if off == 0:
            return row
        return pl.multiple_of(jnp.minimum(row + off, n_kv * sk - size), 8)

    def k_copy(u, j):
        slot = u % nk
        return pltpu.make_async_copy(
            k_hbm.at[pl.ds(dbg(hbm_row(u, kstarts[j]), OFFK, KP[j]), KP[j])],
            kbuf.at[slot, pl.ds(kstarts[j], KP[j])], ksem.at[slot])

    def k_wait(u):
        slot = u % nk
        pltpu.make_async_copy(kbuf.at[slot], kbuf.at[slot], ksem.at[slot]).wait()

    def v_copy(u, j):
        slot = u % nv
        return pltpu.make_async_copy(
            v_hbm.at[pl.ds(dbg(hbm_row(u, vstarts[j]), OFFV, VP[j]), VP[j])],
            vbuf.at[slot, pl.ds(vstarts[j], VP[j])], vsem.at[slot, j])

    def wq_copy(h):
        col = pl.multiple_of(h * hw, hw)
        return pltpu.make_async_copy(wq_hbm.at[:, pl.ds(col, hw)], wqbuf.at[h], wqsem.at[h])

    def wo_copy(h):
        col = pl.multiple_of(h * hw, hw)
        return pltpu.make_async_copy(wot_hbm.at[:, pl.ds(col, hw)], wobuf.at[h], wosem.at[h])

    n_rg = d_model // 8
    n_w16 = d_model // 16
    ffn_per_head = (3 * n_rg) // n_kv
    assert ffn_per_head * n_kv == 3 * n_rg and 2 * n_w16 + ffn_per_head <= upb

    def wq_piece(h, i):
        col = pl.multiple_of(h * hw, hw)
        row = pl.multiple_of(i * 16, 16)
        return pltpu.make_async_copy(wq_hbm.at[pl.ds(row, 16), pl.ds(col, hw)],
                                     wqbuf.at[h, pl.ds(row, 16)], wqsem.at[h])

    def wo_piece(h, i):
        col = pl.multiple_of(h * hw, hw)
        row = pl.multiple_of(i * 16, 16)
        return pltpu.make_async_copy(wot_hbm.at[pl.ds(row, 16), pl.ds(col, hw)],
                                     wobuf.at[h, pl.ds(row, 16)], wosem.at[h])

    def ffn_piece(src, dst, sem, i):
        row = pl.multiple_of(i * 8, 8)
        return pltpu.make_async_copy(src.at[pl.ds(row, 8)], dst.at[pl.ds(row, 8)], sem)

    def wait_all(buf, sem):
        pltpu.make_async_copy(buf, buf, sem).wait()

    def issue_weight_piece(h, r):
        @pl.when(r < 2 * n_w16 + ffn_per_head)
        def _():
            @pl.when(jnp.logical_and(r < n_w16, h < n_kv - 1))
            def _():
                wq_piece(h + 1, r).start(priority=XPRIO)

            @pl.when(jnp.logical_and(r >= n_w16, r < 2 * n_w16))
            def _():
                wo_piece(h, r - n_w16).start(priority=XPRIO)

            f = h * ffn_per_head + r - 2 * n_w16

            @pl.when(r >= 2 * n_w16)
            def _():
                @pl.when(f < n_rg)
                def _():
                    ffn_piece(wg_hbm, wgbuf, msem.at[2], f).start(priority=XPRIO)

                @pl.when(jnp.logical_and(f >= n_rg, f < 2 * n_rg))
                def _():
                    ffn_piece(wu_hbm, wubuf, msem.at[3], f - n_rg).start(priority=XPRIO)

                @pl.when(f >= 2 * n_rg)
                def _():
                    ffn_piece(wdt_hbm, wdbuf, msem.at[4], f - 2 * n_rg).start(priority=XPRIO)

    x_copy = pltpu.make_async_copy(x_hbm, xbuf, msem.at[0])
    wr_copy = pltpu.make_async_copy(wr_hbm, wrbuf, msem.at[1])
    wg_copy = pltpu.make_async_copy(wg_hbm, wgbuf, msem.at[2])
    wu_copy = pltpu.make_async_copy(wu_hbm, wubuf, msem.at[3])
    wd_copy = pltpu.make_async_copy(wdt_hbm, wdbuf, msem.at[4])
    out_copy = pltpu.make_async_copy(obuf, o_hbm, msem.at[5])

    x_copy.start(priority=HI)
    wr_copy.start(priority=HI)
    wq_copy(0).start(priority=HI)
    for u in range(AK + 1):
        for j in range(nkp):
            k_copy(u, j).start(priority=HI)
    for u in range(AV):
        for j in range(ns):
            v_copy(u, j).start(priority=LO)

    x_copy.wait()
    x = xbuf[0].astype(f32)
    mu = jnp.mean(x, axis=1, keepdims=True)
    xc = x - mu
    var = jnp.mean(xc * xc, axis=1, keepdims=True)
    xn = (xc / jnp.sqrt(var + 1e-5)).astype(bf16)
    xn_scr[...] = jnp.broadcast_to(xn, (8, d_model))

    row = jax.lax.broadcasted_iota(jnp.int32, (8, dh), 0)
    top = row < 4

    def make_q(h):
        qf = jnp.dot(xn_scr[...], wqbuf[h], preferred_element_type=f32)
        qh = jnp.where(top, qf[:, :dh], qf[:, dh:]).astype(bf16)
        q_scr[h] = (qh.astype(f32) * (dh ** -0.5)).astype(bf16)

    wq_copy(0).wait()
    make_q(0)
    out_scr[...] = jnp.zeros(out_scr.shape, f32)

    def qk(u, b):
        kk = kbuf[u % nk, pl.ds(b * CB, CB), :]
        return jax.lax.dot_general(q_scr[u // upb], kk, (((1,), (1,)), ((), ())),
                                   preferred_element_type=f32)

    def softmax(u, s_parts, m, l):
        first = (u % upb) == 0
        m_prev = jnp.where(first, NEG, m)
        l_prev = jnp.where(first, 0.0, l)
        s = jnp.concatenate(s_parts, axis=1)
        m_new = jnp.maximum(m_prev, jnp.max(s, axis=1, keepdims=True))
        p = jnp.exp(s - m_new)
        alpha = jnp.exp(m_prev - m_new)
        ps = p[:, 0:128]
        for c in range(1, U // 128):
            ps = ps + p[:, c * 128:(c + 1) * 128]
        return p.astype(bf16), alpha, m_new, alpha * l_prev + ps

    def pv(u, p, b):
        vv = vbuf[u % nv, pl.ds(b * CB, CB), :]
        return jnp.dot(p[:, b * CB:(b + 1) * CB], vv, preferred_element_type=f32)

    k_wait(0)
    s0 = [qk(0, b) for b in range(nb)]
    p0, a0, m0, l0 = softmax(0, s0, jnp.full((8, 1), NEG, f32), jnp.zeros((8, 128), f32))
    acc0 = jnp.zeros((8, dh), f32)

    plan = PLAN if PLAN is not None else _auto_plan(VP, nb)

    def body(u, carry, issue_k, issue_v, has_next):
        p, alpha, m, l, acc = carry
        h = u // upb
        r = u % upb
        s_parts = [None] * nb
        pv_sum = None
        nxt = (p, alpha, m, l)
        for j in range(ns):
            v_copy(u, j).wait()
            if issue_v and VFIRST:
                v_copy(u + AV, j).start(priority=LO)
            if issue_k:
                for jk in range(nkp):
                    if kev[jk] == j:
                        k_copy(u + 1 + AK, jk).start(priority=HI)
            if issue_v and not VFIRST:
                v_copy(u + AV, j).start(priority=LO)
            if SPREAD and j == XEV:
                issue_weight_piece(h, r)
            for item in plan[j]:
                if item[0] == "qk":
                    if has_next:
                        if item[1] == 0:
                            k_wait(u + 1)
                        s_parts[item[1]] = qk(u + 1, item[1])
                elif item[0] == "sm":
                    if has_next:
                        nxt = softmax(u + 1, s_parts, m, l)
                else:
                    res = pv(u, p, item[1])
                    pv_sum = res if pv_sum is None else pv_sum + res
        acc = alpha * acc + pv_sum

        @pl.when(jnp.logical_and(r == 0, not SPREAD))
        def _():
            @pl.when(h < n_kv - 1)
            def _():
                wq_copy(h + 1).start(priority=LO)
            wo_copy(h).start(priority=LO)

            @pl.when(h == 0)
            def _():
                wg_copy.start(priority=LO)

            @pl.when(h == 1)
            def _():
                wu_copy.start(priority=LO)

            @pl.when(h == 2)
            def _():
                wd_copy.start(priority=LO)

        @pl.when(jnp.logical_and(r == upb // 2, h < n_kv - 1))
        def _():
            wait_all(wqbuf.at[h + 1], wqsem.at[h + 1])
            make_q(h + 1)

        @pl.when(jnp.logical_and(r == (3 * upb) // 4, h == n_kv - 1))
        def _():
            wait_all(wgbuf, msem.at[2])
            wait_all(wubuf, msem.at[3])
            wait_all(wdbuf, msem.at[4])
            wr_copy.wait()
            xb = xn_scr[...]
            g = jnp.dot(xb, wgbuf[...], preferred_element_type=f32).astype(bf16).astype(f32)
            up = jnp.dot(xb, wubuf[...], preferred_element_type=f32).astype(bf16).astype(f32)
            g = (g * jax.nn.sigmoid(g)).astype(bf16)
            hid = (g.astype(f32) * up).astype(bf16)
            y = jax.lax.dot_general(hid, wdbuf[...], (((1,), (1,)), ((), ())),
                                    preferred_element_type=f32)
            xf = xb.astype(f32)
            wr = wrbuf[...].astype(f32).reshape(1, d_model)
            rs = jax.nn.sigmoid(jnp.sum(xf * wr, axis=1, keepdims=True))
            rows = jax.lax.broadcasted_iota(jnp.int32, (8, d_model), 0)
            base = xf + xf * 0.0 + y * rs
            out_scr[...] += jnp.where(rows == 0, base, 0.0)

        @pl.when(r == upb - 1)
        def _():
            o = acc / jnp.sum(l, axis=1, keepdims=True)
            sel0 = row == 0
            sel1 = row == 4
            lhs = jnp.concatenate([jnp.where(sel0, o, 0.0), jnp.where(sel1, o, 0.0)],
                                  axis=1).astype(bf16)
            wait_all(wobuf.at[h], wosem.at[h])
            out_scr[...] += jax.lax.dot_general(lhs, wobuf[h], (((1,), (1,)), ((), ())),
                                                preferred_element_type=f32)
        return nxt + (acc,)

    carry = (p0, a0, m0, l0, acc0)
    n1 = n_units - max(AV, AK + 1)
    carry = jax.lax.fori_loop(0, n1, lambda u, c: body(u, c, True, True, True), carry)
    if AV > AK + 1:
        carry = jax.lax.fori_loop(n1, n_units - AK - 1,
                                  lambda u, c: body(u, c, True, False, True), carry)
    elif AK + 1 > AV:
        carry = jax.lax.fori_loop(n1, n_units - AV,
                                  lambda u, c: body(u, c, False, True, True), carry)
    n2 = n_units - min(AV, AK + 1)
    carry = jax.lax.fori_loop(n2, n_units - 1,
                              lambda u, c: body(u, c, False, False, True), carry)
    body(n_units - 1, carry, False, False, False)

    res = jnp.sum(out_scr[...], axis=0, keepdims=True) + xbuf[0].astype(f32)
    obuf[0] = res.astype(obuf.dtype)
    out_copy.start()
    out_copy.wait()


@jax.jit
def pallas_parallel_sum__gqa_block_cached__moe_arch_mod__decode_kernel(
    A_x: jax.Array,
    A_k_cache: jax.Array,
    A_v_cache: jax.Array,
    A_wq: jax.Array,
    A_wo: jax.Array,
    B_x: jax.Array,
    B_w_r: jax.Array,
    B_w_gate: jax.Array,
    B_w_up: jax.Array,
    B_w_down: jax.Array,
):
    del B_x
    _, n_kv, sk, dh = A_k_cache.shape
    d_model = A_x.shape[-1]
    hq = A_wq.shape[1] // dh
    rep = hq // n_kv
    assert rep == 2 and A_x.shape == (1, 1, d_model)
    ffn = B_w_gate.shape[1]
    hw = rep * dh
    ns = len(VP)
    bf16 = jnp.bfloat16

    k2 = A_k_cache.reshape(n_kv * sk, dh)
    v2 = A_v_cache.reshape(n_kv * sk, dh)
    wot = A_wo.T
    wdt = B_w_down.T

    kernel = functools.partial(_kernel, n_kv=n_kv, sk=sk, dh=dh, d_model=d_model, rep=rep)
    return pl.pallas_call(
        kernel,
        out_shape=jax.ShapeDtypeStruct((1, 1, d_model), A_x.dtype),
        in_specs=[pl.BlockSpec(memory_space=pl.ANY)] * 9,
        out_specs=pl.BlockSpec(memory_space=pl.ANY),
        scratch_shapes=[
            pltpu.VMEM((1, 1, d_model), bf16),
            pltpu.VMEM((d_model,), bf16),
            pltpu.VMEM((1, 1, d_model), bf16),
            pltpu.VMEM((PADK // 4 + 1, 8, 128), jnp.float32),
            pltpu.VMEM((AK + 1, U, dh), bf16),
            pltpu.VMEM((PADV // 4 + 1, 8, 128), jnp.float32),
            pltpu.VMEM((AV + 1, U, dh), bf16),
            pltpu.VMEM((n_kv, d_model, hw), bf16),
            pltpu.VMEM((n_kv, d_model, hw), bf16),
            pltpu.VMEM((d_model, ffn), bf16),
            pltpu.VMEM((d_model, ffn), bf16),
            pltpu.VMEM((d_model, ffn), bf16),
            pltpu.VMEM((8, d_model), bf16),
            pltpu.VMEM((n_kv, 8, dh), bf16),
            pltpu.VMEM((8, d_model), jnp.float32),
            pltpu.SemaphoreType.DMA((AK + 1,)),
            pltpu.SemaphoreType.DMA((AV + 1, ns)),
            pltpu.SemaphoreType.DMA((n_kv,)),
            pltpu.SemaphoreType.DMA((n_kv,)),
            pltpu.SemaphoreType.DMA((6,)),
        ],
        compiler_params=pltpu.CompilerParams(vmem_limit_bytes=64 * 1024 * 1024,
                                             disable_bounds_checks=NO_BOUNDS),
    )(A_x, k2, v2, A_wq, wot, B_w_r, B_w_gate, B_w_up, wdt)
```

```python
import functools

import jax
import jax.numpy as jnp
import jax.experimental.pallas as pl
import jax.experimental.pallas.tpu as pltpu


HI = 0
LO = 1

U = 512
KP = (56, 128, 24, 104, 120, 80)
VP = (48, 120, 16, 112, 128, 88)
KEV = (0, 1, 3, 3, 4, 5)
PLAN = None
AK = 3
AV = 7
XEV = 1
CB = 256
TCB = 256
NEG = -1e30
DBG_SKIP = ()


def _default_plan(ns, nb):
    plan = [[] for _ in range(ns)]
    plan[0] = [("qk", b) for b in range(nb)]
    plan[1] = [("sm",)]
    plan[ns - 1] = [("pv", b) for b in range(nb)]
    return plan


def _kernel(x_hbm, k_hbm, v_hbm, wq_hbm, wot_hbm, wr_hbm, wg_hbm, wu_hbm, wdt_hbm,
            o_hbm,
            xbuf, wrbuf, obuf, kbuf, vbuf, wqbuf, wobuf, wgbuf, wubuf, wdbuf,
            xn_scr, q_scr, out_scr,
            ksem, vsem, wqsem, wosem, msem,
            *, n_kv, sk, dh, d_model):
    ns = len(VP)
    nkp = len(KP)
    kev = list(KEV) if KEV is not None else list(range(nkp))
    assert len(kev) == nkp and max(kev) < ns and sum(KP) == U and sum(VP) == U
    kstarts = [sum(KP[:j]) for j in range(nkp)]
    vstarts = [sum(VP[:j]) for j in range(ns)]
    nb = U // CB
    upb = sk // U
    n_units = n_kv * upb
    nk = AK + 1
    nv = AV + 1
    hw = 2 * dh
    f32 = jnp.float32
    bf16 = jnp.bfloat16
    nt_dims = (((1,), (1,)), ((), ()))

    def k_copy(u, j):
        slot = u % nk
        return pltpu.make_async_copy(
            k_hbm.at[pl.ds(u * U + kstarts[j], KP[j])],
            kbuf.at[slot, pl.ds(kstarts[j], KP[j])], ksem.at[slot])

    def v_copy(u, j):
        slot = u % nv
        return pltpu.make_async_copy(
            v_hbm.at[pl.ds(u * U + vstarts[j], VP[j])],
            vbuf.at[slot, pl.ds(vstarts[j], VP[j])], vsem.at[slot, j])

    def wait_all(buf, sem):
        pltpu.make_async_copy(buf, buf, sem).wait()

    def k_wait(u):
        wait_all(kbuf.at[u % nk], ksem.at[u % nk])

    n_rg = d_model // 8
    n_w16 = d_model // 16
    ffn_per_head = (3 * n_rg) // n_kv
    n_extra = 2 * n_w16 + ffn_per_head
    assert ffn_per_head * n_kv == 3 * n_rg and n_extra <= upb // 2 + upb // 8

    def head_piece(src, dst, sem, h, i):
        col = pl.multiple_of(h * hw, hw)
        row = pl.multiple_of(i * 16, 16)
        return pltpu.make_async_copy(src.at[pl.ds(row, 16), pl.ds(col, hw)],
                                     dst.at[h, pl.ds(row, 16)], sem.at[h])

    def ffn_piece(src, dst, sem, i):
        row = pl.multiple_of(i * 8, 8)
        return pltpu.make_async_copy(src.at[pl.ds(row, 8)], dst.at[pl.ds(row, 8)], sem)

    def issue_weight_piece(h, r):
        @pl.when(r < n_extra)
        def _():
            @pl.when(jnp.logical_and(r < n_w16, h < n_kv - 1))
            def _():
                head_piece(wq_hbm, wqbuf, wqsem, h + 1, r).start(priority=HI)

            @pl.when(jnp.logical_and(r >= n_w16, r < 2 * n_w16))
            def _():
                head_piece(wot_hbm, wobuf, wosem, h, r - n_w16).start(priority=HI)

            f = h * ffn_per_head + r - 2 * n_w16

            @pl.when(r >= 2 * n_w16)
            def _():
                @pl.when(f < n_rg)
                def _():
                    ffn_piece(wg_hbm, wgbuf, msem.at[2], f).start(priority=HI)

                @pl.when(jnp.logical_and(f >= n_rg, f < 2 * n_rg))
                def _():
                    ffn_piece(wu_hbm, wubuf, msem.at[3], f - n_rg).start(priority=HI)

                @pl.when(f >= 2 * n_rg)
                def _():
                    ffn_piece(wdt_hbm, wdbuf, msem.at[4], f - 2 * n_rg).start(priority=HI)

    x_copy = pltpu.make_async_copy(x_hbm, xbuf, msem.at[0])
    wr_copy = pltpu.make_async_copy(wr_hbm, wrbuf, msem.at[1])
    wq0_copy = pltpu.make_async_copy(wq_hbm.at[:, pl.ds(0, hw)], wqbuf.at[0], wqsem.at[0])
    out_copy = pltpu.make_async_copy(obuf, o_hbm, msem.at[5])

    x_copy.start(priority=HI)
    wr_copy.start(priority=HI)
    wq0_copy.start(priority=HI)
    for u in range(AK + 1):
        for j in range(nkp):
            k_copy(u, j).start(priority=HI)
    for u in range(AV):
        for j in range(ns):
            v_copy(u, j).start(priority=LO)

    x_copy.wait()
    x = xbuf[0].astype(f32)
    mu = jnp.mean(x, axis=1, keepdims=True)
    xc = x - mu
    var = jnp.mean(xc * xc, axis=1, keepdims=True)
    xn = (xc / jnp.sqrt(var + 1e-5)).astype(bf16)
    xn_scr[...] = jnp.broadcast_to(xn, (8, d_model))

    row = jax.lax.broadcasted_iota(jnp.int32, (8, dh), 0)
    top = row < 4

    def make_q(h):
        qf = jnp.dot(xn_scr[...], wqbuf[h], preferred_element_type=f32)
        qh = jnp.where(top, qf[:, :dh], qf[:, dh:]).astype(bf16)
        q_scr[h] = (qh.astype(f32) * (dh ** -0.5)).astype(bf16)

    wq0_copy.wait()
    make_q(0)
    out_scr[...] = jnp.zeros(out_scr.shape, f32)

    def qk(u, b):
        kk = kbuf[u % nk, pl.ds(b * CB, CB), :]
        return jax.lax.dot_general(q_scr[u // upb], kk, nt_dims, preferred_element_type=f32)

    def softmax(u, s_parts, m, l):
        first = (u % upb) == 0
        m_prev = jnp.where(first, NEG, m)
        l_prev = jnp.where(first, 0.0, l)
        s = jnp.concatenate(s_parts, axis=1)
        m_new = jnp.maximum(m_prev, jnp.max(s, axis=1, keepdims=True))
        p = jnp.exp(s - m_new)
        alpha = jnp.exp(m_prev - m_new)
        ps = p[:, 0:128]
        for c in range(1, U // 128):
            ps = ps + p[:, c * 128:(c + 1) * 128]
        return p.astype(bf16), alpha, m_new, alpha * l_prev + ps

    def pv(u, p, start, size):
        vv = vbuf[u % nv, pl.ds(start, size), :]
        return jnp.dot(p[:, start:start + size], vv, preferred_element_type=f32)

    def project(h, o):
        lhs = jnp.concatenate([jnp.where(row == 0, o, 0.0), jnp.where(row == 4, o, 0.0)],
                              axis=1).astype(bf16)
        return jax.lax.dot_general(lhs, wobuf[h], nt_dims, preferred_element_type=f32)

    def ffn():
        wait_all(wgbuf, msem.at[2])
        wait_all(wubuf, msem.at[3])
        wait_all(wdbuf, msem.at[4])
        wr_copy.wait()
        if 'ffn' in DBG_SKIP:
            return
        xb = xn_scr[...]
        g = jnp.dot(xb, wgbuf[...], preferred_element_type=f32).astype(bf16).astype(f32)
        up = jnp.dot(xb, wubuf[...], preferred_element_type=f32).astype(bf16).astype(f32)
        g = (g * jax.nn.sigmoid(g)).astype(bf16)
        hid = (g.astype(f32) * up).astype(bf16)
        y = jax.lax.dot_general(hid, wdbuf[...], nt_dims, preferred_element_type=f32)
        xf = xb.astype(f32)
        wr = wrbuf[...].astype(f32).reshape(1, d_model)
        rs = jax.nn.sigmoid(jnp.sum(xf * wr, axis=1, keepdims=True))
        rows = jax.lax.broadcasted_iota(jnp.int32, (8, d_model), 0)
        base = xbuf[0].astype(f32) + xf + xf * 0.0 + y * rs
        out_scr[...] += jnp.where(rows == 0, base, 0.0)

    k_wait(0)
    s0 = [qk(0, b) for b in range(nb)]
    p0, a0, m0, l0 = softmax(0, s0, jnp.full((8, 1), NEG, f32), jnp.zeros((8, 128), f32))
    acc0 = jnp.zeros((8, dh), f32)

    plan = PLAN if PLAN is not None else _default_plan(ns, nb)

    def body(u, carry, issue_k, issue_v, main):
        p, alpha, m, l, acc = carry
        h = u // upb
        r = u % upb
        s_parts = [None] * nb
        pv_sum = None
        nxt = None
        for j in range(ns):
            v_copy(u, j).wait()
            if issue_k:
                for jk in range(nkp):
                    if kev[jk] == j:
                        k_copy(u + 1 + AK, jk).start(priority=HI)
            if issue_v:
                v_copy(u + AV, j).start(priority=LO)
            if main and j == XEV:
                issue_weight_piece(h, r)
            for item in plan[j]:
                if item[0] == "qk":
                    if item[1] == 0:
                        k_wait(u + 1)
                    s_parts[item[1]] = qk(u + 1, item[1])
                elif item[0] == "sm":
                    nxt = softmax(u + 1, s_parts, m, l)
                else:
                    res = pv(u, p, item[1] * CB, CB)
                    pv_sum = res if pv_sum is None else pv_sum + res
        acc = alpha * acc + pv_sum

        if main:
            @pl.when(jnp.logical_and(r == upb // 2, h < n_kv - 1))
            def _():
                wait_all(wqbuf.at[h + 1], wqsem.at[h + 1])
                if 'q' in DBG_SKIP:
                    q_scr[h + 1] = q_scr[0]
                else:
                    make_q(h + 1)

            @pl.when(u == n_units - upb // 4)
            def _():
                ffn()

            @pl.when(r == upb - 1)
            def _():
                o = acc / jnp.sum(l, axis=1, keepdims=True)
                wait_all(wobuf.at[h], wosem.at[h])
                if 'fin' not in DBG_SKIP:
                    out_scr[...] += project(h, o)
        return nxt + (acc,)

    carry = (p0, a0, m0, l0, acc0)
    n1 = n_units - max(AV, AK + 1)
    assert n1 > n_units - upb // 4
    carry = jax.lax.fori_loop(0, n1, lambda u, c: body(u, c, True, True, True), carry)
    if AV > AK + 1:
        carry = jax.lax.fori_loop(n1, n_units - AK - 1,
                                  lambda u, c: body(u, c, True, False, False), carry)
    elif AK + 1 > AV:
        carry = jax.lax.fori_loop(n1, n_units - AV,
                                  lambda u, c: body(u, c, False, True, False), carry)
    n2 = n_units - min(AV, AK + 1)
    carry = jax.lax.fori_loop(n2, n_units - 1,
                              lambda u, c: body(u, c, False, False, False), carry)

    p, alpha, m, l, acc = carry
    u = n_units - 1
    wait_all(wobuf.at[n_kv - 1], wosem.at[n_kv - 1])
    rinv = 1.0 / jnp.sum(l, axis=1, keepdims=True)
    acc = alpha * acc
    done = 0
    for j in range(ns):
        v_copy(u, j).wait()
        end = vstarts[j] + VP[j]
        while done + TCB <= end:
            acc = acc + pv(u, p, done, TCB)
            done += TCB
    tot = out_scr[...] + project(n_kv - 1, acc * rinv)
    obuf[0] = jnp.sum(tot, axis=0, keepdims=True).astype(obuf.dtype)
    out_copy.start()
    out_copy.wait()


@jax.jit
def pallas_parallel_sum__gqa_block_cached__moe_arch_mod__decode_kernel(
    A_x: jax.Array,
    A_k_cache: jax.Array,
    A_v_cache: jax.Array,
    A_wq: jax.Array,
    A_wo: jax.Array,
    B_x: jax.Array,
    B_w_r: jax.Array,
    B_w_gate: jax.Array,
    B_w_up: jax.Array,
    B_w_down: jax.Array,
):
    del B_x
    _, n_kv, sk, dh = A_k_cache.shape
    d_model = A_x.shape[-1]
    assert A_wq.shape[1] == 2 * n_kv * dh and A_x.shape == (1, 1, d_model)
    ffn = B_w_gate.shape[1]
    hw = 2 * dh
    ns = len(VP)
    bf16 = jnp.bfloat16

    k2 = A_k_cache.reshape(n_kv * sk, dh)
    v2 = A_v_cache.reshape(n_kv * sk, dh)
    wot = A_wo.T
    wdt = B_w_down.T

    kernel = functools.partial(_kernel, n_kv=n_kv, sk=sk, dh=dh, d_model=d_model)
    return pl.pallas_call(
        kernel,
        out_shape=jax.ShapeDtypeStruct((1, 1, d_model), A_x.dtype),
        in_specs=[pl.BlockSpec(memory_space=pl.ANY)] * 9,
        out_specs=pl.BlockSpec(memory_space=pl.ANY),
        scratch_shapes=[
            pltpu.VMEM((1, 1, d_model), bf16),
            pltpu.VMEM((d_model,), bf16),
            pltpu.VMEM((1, 1, d_model), bf16),
            pltpu.VMEM((AK + 1, U, dh), bf16),
            pltpu.VMEM((AV + 1, U, dh), bf16),
            pltpu.VMEM((n_kv, d_model, hw), bf16),
            pltpu.VMEM((n_kv, d_model, hw), bf16),
            pltpu.VMEM((d_model, ffn), bf16),
            pltpu.VMEM((d_model, ffn), bf16),
            pltpu.VMEM((d_model, ffn), bf16),
            pltpu.VMEM((8, d_model), bf16),
            pltpu.VMEM((n_kv, 8, dh), bf16),
            pltpu.VMEM((8, d_model), jnp.float32),
            pltpu.SemaphoreType.DMA((AK + 1,)),
            pltpu.SemaphoreType.DMA((AV + 1, ns)),
            pltpu.SemaphoreType.DMA((n_kv,)),
            pltpu.SemaphoreType.DMA((n_kv,)),
            pltpu.SemaphoreType.DMA((6,)),
        ],
        compiler_params=pltpu.CompilerParams(vmem_limit_bytes=64 * 1024 * 1024,
                                             disable_bounds_checks=True),
    )(A_x, k2, v2, A_wq, wot, B_w_r, B_w_gate, B_w_up, wdt)
```

```python
import functools

import jax
import jax.numpy as jnp
import jax.experimental.pallas as pl
import jax.experimental.pallas.tpu as pltpu


HI = 0
LO = 1

U = 512
KP = (56, 128, 24, 104, 120, 80)
VP = (48, 120, 16, 120, 120, 88)
KEV = (0, 1, 3, 3, 4, 5)
PLAN = None
AK = 3
AV = 7
XEV = 1
CB = 256
TCB = 256
NEG = -1e30
NO_SEM_CHECK = True
SKIP_BAR = False
DBG_SKIP = ()
DBG_UPB = None
DBG_NKV = None


def _default_plan(ns, nb):
    plan = [[] for _ in range(ns)]
    plan[0] = [("qk", b) for b in range(nb)]
    plan[1] = [("sm",)]
    plan[ns - 1] = [("pv", b) for b in range(nb)]
    return plan


def _kernel(x_hbm, k_hbm, v_hbm, wq_hbm, wot_hbm, wr_hbm, wg_hbm, wu_hbm, wdt_hbm,
            o_hbm,
            xbuf, wrbuf, obuf, kbuf, vbuf, wqbuf, wobuf, wgbuf, wubuf, wdbuf,
            xn_scr, q_scr, out_scr,
            ksem, vsem, wqsem, wosem, msem,
            *, n_kv, sk, dh, d_model):
    ns = len(VP)
    nkp = len(KP)
    kev = list(KEV) if KEV is not None else list(range(nkp))
    assert len(kev) == nkp and max(kev) < ns and sum(KP) == U and sum(VP) == U
    kstarts = [sum(KP[:j]) for j in range(nkp)]
    vstarts = [sum(VP[:j]) for j in range(ns)]
    nb = U // CB
    upb = sk // U
    upb_full = upb
    if DBG_UPB is not None:
        upb = DBG_UPB
    n_units = n_kv * upb
    if DBG_NKV is not None:
        n_units = DBG_NKV * upb
    nk = AK + 1
    nv = AV + 1
    hw = 2 * dh
    f32 = jnp.float32
    bf16 = jnp.bfloat16
    nt_dims = (((1,), (1,)), ((), ()))

    def urow(u):
        if upb == upb_full:
            return u * U
        return ((u // upb) * upb_full + u % upb) * U

    def k_copy(u, j):
        slot = u % nk
        return pltpu.make_async_copy(
            k_hbm.at[pl.ds(urow(u) + kstarts[j], KP[j])],
            kbuf.at[slot, pl.ds(kstarts[j], KP[j])], ksem.at[slot])

    def v_copy(u, j):
        slot = u % nv
        return pltpu.make_async_copy(
            v_hbm.at[pl.ds(urow(u) + vstarts[j], VP[j])],
            vbuf.at[slot, pl.ds(vstarts[j], VP[j])], vsem.at[slot, j])

    def wait_all(buf, sem, weights=False):
        if weights and 'now' in DBG_SKIP:
            return
        pltpu.make_async_copy(buf, buf, sem).wait()

    def k_wait(u):
        wait_all(kbuf.at[u % nk], ksem.at[u % nk])

    n_rg = d_model // 8
    n_w16 = d_model // 16
    ffn_per_head = (3 * n_rg) // n_kv
    n_extra = 2 * n_w16 + ffn_per_head
    assert ffn_per_head * n_kv == 3 * n_rg and (n_extra <= upb - upb // 4 or 'now' in DBG_SKIP)

    def head_piece(src, dst, sem, h, i):
        col = pl.multiple_of(h * hw, hw)
        row = pl.multiple_of(i * 16, 16)
        return pltpu.make_async_copy(src.at[pl.ds(row, 16), pl.ds(col, hw)],
                                     dst.at[h, pl.ds(row, 16)], sem.at[h])

    def ffn_piece(src, dst, sem, i):
        row = pl.multiple_of(i * 8, 8)
        return pltpu.make_async_copy(src.at[pl.ds(row, 8)], dst.at[pl.ds(row, 8)], sem)

    def issue_weight_piece(h, r):
        @pl.when(r < n_extra)
        def _():
            @pl.when(jnp.logical_and(r < n_w16, h < n_kv - 1))
            def _():
                head_piece(wq_hbm, wqbuf, wqsem, h + 1, r).start(priority=HI)

            @pl.when(jnp.logical_and(r >= n_w16, r < 2 * n_w16))
            def _():
                head_piece(wot_hbm, wobuf, wosem, h, r - n_w16).start(priority=HI)

            f = h * ffn_per_head + r - 2 * n_w16

            @pl.when(r >= 2 * n_w16)
            def _():
                @pl.when(f < n_rg)
                def _():
                    ffn_piece(wg_hbm, wgbuf, msem.at[2], f).start(priority=HI)

                @pl.when(jnp.logical_and(f >= n_rg, f < 2 * n_rg))
                def _():
                    ffn_piece(wu_hbm, wubuf, msem.at[3], f - n_rg).start(priority=HI)

                @pl.when(f >= 2 * n_rg)
                def _():
                    ffn_piece(wdt_hbm, wdbuf, msem.at[4], f - 2 * n_rg).start(priority=HI)

    x_copy = pltpu.make_async_copy(x_hbm, xbuf, msem.at[0])
    wr_copy = pltpu.make_async_copy(wr_hbm, wrbuf, msem.at[1])
    wq0_copy = pltpu.make_async_copy(wq_hbm.at[:, pl.ds(0, hw)], wqbuf.at[0], wqsem.at[0])
    out_copy = pltpu.make_async_copy(obuf, o_hbm, msem.at[5])

    x_copy.start(priority=HI)
    wr_copy.start(priority=HI)
    wq0_copy.start(priority=HI)
    for u in range(AK + 1):
        for j in range(nkp):
            k_copy(u, j).start(priority=HI)
    for u in range(AV):
        for j in range(ns):
            v_copy(u, j).start(priority=LO)

    x_copy.wait()
    x = xbuf[0].astype(f32)
    mu = jnp.mean(x, axis=1, keepdims=True)
    xc = x - mu
    var = jnp.mean(xc * xc, axis=1, keepdims=True)
    xn = (xc / jnp.sqrt(var + 1e-5)).astype(bf16)
    xn_scr[...] = jnp.broadcast_to(xn, (8, d_model))

    row = jax.lax.broadcasted_iota(jnp.int32, (8, dh), 0)
    top = row < 4

    def make_q(h):
        qf = jnp.dot(xn_scr[...], wqbuf[h], preferred_element_type=f32)
        qh = jnp.where(top, qf[:, :dh], qf[:, dh:]).astype(bf16)
        q_scr[h] = (qh.astype(f32) * (dh ** -0.5)).astype(bf16)

    if 'pro' in DBG_SKIP:
        q_scr[0] = jnp.zeros((8, dh), bf16)
    else:
        wq0_copy.wait()
        make_q(0)
    out_scr[...] = jnp.zeros(out_scr.shape, f32)

    def qk(u, b):
        kk = kbuf[u % nk, pl.ds(b * CB, CB), :]
        return jax.lax.dot_general(q_scr[u // upb], kk, nt_dims, preferred_element_type=f32)

    def softmax(u, s_parts, m, l):
        first = (u % upb) == 0
        m_prev = jnp.where(first, NEG, m)
        l_prev = jnp.where(first, 0.0, l)
        s = jnp.concatenate(s_parts, axis=1)
        m_new = jnp.maximum(m_prev, jnp.max(s, axis=1, keepdims=True))
        p = jnp.exp(s - m_new)
        alpha = jnp.exp(m_prev - m_new)
        ps = p[:, 0:128]
        for c in range(1, U // 128):
            ps = ps + p[:, c * 128:(c + 1) * 128]
        return p.astype(bf16), alpha, m_new, alpha * l_prev + ps

    def pv(u, p, start, size):
        vv = vbuf[u % nv, pl.ds(start, size), :]
        return jnp.dot(p[:, start:start + size], vv, preferred_element_type=f32)

    def project(h, o):
        lhs = jnp.concatenate([jnp.where(row == 0, o, 0.0), jnp.where(row == 4, o, 0.0)],
                              axis=1).astype(bf16)
        return jax.lax.dot_general(lhs, wobuf[h], nt_dims, preferred_element_type=f32)

    def ffn():
        wait_all(wgbuf, msem.at[2], True)
        wait_all(wubuf, msem.at[3], True)
        wait_all(wdbuf, msem.at[4], True)
        wr_copy.wait()
        if 'ffn' in DBG_SKIP:
            return
        xb = xn_scr[...]
        g = jnp.dot(xb, wgbuf[...], preferred_element_type=f32).astype(bf16).astype(f32)
        up = jnp.dot(xb, wubuf[...], preferred_element_type=f32).astype(bf16).astype(f32)
        g = (g * jax.nn.sigmoid(g)).astype(bf16)
        hid = (g.astype(f32) * up).astype(bf16)
        y = jax.lax.dot_general(hid, wdbuf[...], nt_dims, preferred_element_type=f32)
        xf = xb.astype(f32)
        wr = wrbuf[...].astype(f32).reshape(1, d_model)
        rs = jax.nn.sigmoid(jnp.sum(xf * wr, axis=1, keepdims=True))
        rows = jax.lax.broadcasted_iota(jnp.int32, (8, d_model), 0)
        base = xbuf[0].astype(f32) + xf + xf * 0.0 + y * rs
        out_scr[...] += jnp.where(rows == 0, base, 0.0)

    k_wait(0)
    s0 = [qk(0, b) for b in range(nb)]
    p0, a0, m0, l0 = softmax(0, s0, jnp.full((8, 1), NEG, f32), jnp.zeros((8, 128), f32))
    acc0 = jnp.zeros((8, dh), f32)

    plan = PLAN if PLAN is not None else _default_plan(ns, nb)

    def body(u, carry, issue_k, issue_v, main):
        p, alpha, m, l, acc = carry
        h = u // upb
        r = u % upb
        s_parts = [None] * nb
        pv_sum = None
        nxt = None
        for j in range(ns):
            v_copy(u, j).wait()
            if issue_k:
                for jk in range(nkp):
                    if kev[jk] == j:
                        k_copy(u + 1 + AK, jk).start(priority=HI)
            if issue_v:
                v_copy(u + AV, j).start(priority=LO)
            if main and j == XEV and 'now' not in DBG_SKIP:
                issue_weight_piece(h, r)
            for item in plan[j]:
                if item[0] == "qk":
                    if item[1] == 0:
                        k_wait(u + 1)
                    s_parts[item[1]] = qk(u + 1, item[1])
                elif item[0] == "sm":
                    nxt = softmax(u + 1, s_parts, m, l)
                else:
                    res = pv(u, p, item[1] * CB, CB)
                    pv_sum = res if pv_sum is None else pv_sum + res
        acc = alpha * acc + pv_sum

        if main:
            @pl.when(jnp.logical_and(r == upb // 2, h < n_kv - 1))
            def _():
                wait_all(wqbuf.at[h + 1], wqsem.at[h + 1], True)
                if 'q' in DBG_SKIP:
                    q_scr[h + 1] = q_scr[0]
                else:
                    make_q(h + 1)

            @pl.when(u == (n_units - upb // 4 if 'now' not in DBG_SKIP else 2))
            def _():
                ffn()

            @pl.when(r == upb - 1)
            def _():
                o = acc / jnp.sum(l, axis=1, keepdims=True)
                wait_all(wobuf.at[h], wosem.at[h], True)
                if 'fin' not in DBG_SKIP:
                    out_scr[...] += project(h, o)
        return nxt + (acc,)

    carry = (p0, a0, m0, l0, acc0)
    n1 = n_units - max(AV, AK + 1)
    assert n1 > n_units - upb // 4 or 'now' in DBG_SKIP
    carry = jax.lax.fori_loop(0, n1, lambda u, c: body(u, c, True, True, True), carry)
    if AV > AK + 1:
        carry = jax.lax.fori_loop(n1, n_units - AK - 1,
                                  lambda u, c: body(u, c, True, False, False), carry)
    elif AK + 1 > AV:
        carry = jax.lax.fori_loop(n1, n_units - AV,
                                  lambda u, c: body(u, c, False, True, False), carry)
    n2 = n_units - min(AV, AK + 1)
    carry = jax.lax.fori_loop(n2, n_units - 1,
                              lambda u, c: body(u, c, False, False, False), carry)

    if 'pro' in DBG_SKIP:
        wq0_copy.wait()
    p, alpha, m, l, acc = carry
    u = n_units - 1
    wait_all(wobuf.at[n_kv - 1], wosem.at[n_kv - 1], True)
    rinv = 1.0 / jnp.sum(l, axis=1, keepdims=True)
    acc = alpha * acc
    done = 0
    for j in range(ns):
        v_copy(u, j).wait()
        end = vstarts[j] + VP[j]
        while done + TCB <= end and 'tail' not in DBG_SKIP:
            acc = acc + pv(u, p, done, TCB)
            done += TCB
    if 'tail' in DBG_SKIP:
        tot = out_scr[...]
    else:
        tot = out_scr[...] + project(n_kv - 1, acc * rinv)
    obuf[0] = jnp.sum(tot, axis=0, keepdims=True).astype(obuf.dtype)
    out_copy.start()
    out_copy.wait()


@jax.jit
def pallas_parallel_sum__gqa_block_cached__moe_arch_mod__decode_kernel(
    A_x: jax.Array,
    A_k_cache: jax.Array,
    A_v_cache: jax.Array,
    A_wq: jax.Array,
    A_wo: jax.Array,
    B_x: jax.Array,
    B_w_r: jax.Array,
    B_w_gate: jax.Array,
    B_w_up: jax.Array,
    B_w_down: jax.Array,
):
    del B_x
    _, n_kv, sk, dh = A_k_cache.shape
    d_model = A_x.shape[-1]
    assert A_wq.shape[1] == 2 * n_kv * dh and A_x.shape == (1, 1, d_model)
    ffn = B_w_gate.shape[1]
    hw = 2 * dh
    ns = len(VP)
    bf16 = jnp.bfloat16

    k2 = A_k_cache.reshape(n_kv * sk, dh)
    v2 = A_v_cache.reshape(n_kv * sk, dh)
    wot = A_wo.T
    wdt = B_w_down.T

    kernel = functools.partial(_kernel, n_kv=n_kv, sk=sk, dh=dh, d_model=d_model)
    return pl.pallas_call(
        kernel,
        out_shape=jax.ShapeDtypeStruct((1, 1, d_model), A_x.dtype),
        in_specs=[pl.BlockSpec(memory_space=pl.ANY)] * 9,
        out_specs=pl.BlockSpec(memory_space=pl.ANY),
        scratch_shapes=[
            pltpu.VMEM((1, 1, d_model), bf16),
            pltpu.VMEM((d_model,), bf16),
            pltpu.VMEM((1, 1, d_model), bf16),
            pltpu.VMEM((AK + 1, U, dh), bf16),
            pltpu.VMEM((AV + 1, U, dh), bf16),
            pltpu.VMEM((n_kv, d_model, hw), bf16),
            pltpu.VMEM((n_kv, d_model, hw), bf16),
            pltpu.VMEM((d_model, ffn), bf16),
            pltpu.VMEM((d_model, ffn), bf16),
            pltpu.VMEM((d_model, ffn), bf16),
            pltpu.VMEM((8, d_model), bf16),
            pltpu.VMEM((n_kv, 8, dh), bf16),
            pltpu.VMEM((8, d_model), jnp.float32),
            pltpu.SemaphoreType.DMA((AK + 1,)),
            pltpu.SemaphoreType.DMA((AV + 1, ns)),
            pltpu.SemaphoreType.DMA((n_kv,)),
            pltpu.SemaphoreType.DMA((n_kv,)),
            pltpu.SemaphoreType.DMA((6,)),
        ],
        compiler_params=pltpu.CompilerParams(vmem_limit_bytes=64 * 1024 * 1024,
                                             disable_bounds_checks=True,
                                             disable_semaphore_checks=NO_SEM_CHECK,
                                             skip_device_barrier=SKIP_BAR),
    )(A_x, k2, v2, A_wq, wot, B_w_r, B_w_gate, B_w_up, wdt)
```

```python
import functools

import jax
import jax.numpy as jnp
import jax.experimental.pallas as pl
import jax.experimental.pallas.tpu as pltpu


HI = 0
LO = 1

U = 512
KP = (56, 128, 128, 120, 80)
KEV = (0, 1, 3, 4, 5)
VP = (48, 120, 16, 120, 120, 88)
AK = 3
AV = 7
XEV = 1
CB = 256
NEG = -1e30


def _kernel(x_hbm, k_hbm, v_hbm, wq_hbm, wot_hbm, wr_hbm, wg_hbm, wu_hbm, wdt_hbm,
            o_hbm,
            xbuf, wrbuf, obuf, kbuf, vbuf, wqbuf, wobuf, wgbuf, wubuf, wdbuf,
            xn_scr, q_scr, out_scr,
            ksem, vsem, wqsem, wosem, msem,
            *, n_kv, sk, dh, d_model):
    ns = len(VP)
    nkp = len(KP)
    assert len(KEV) == nkp and max(KEV) < ns and sum(KP) == U and sum(VP) == U
    kstarts = [sum(KP[:j]) for j in range(nkp)]
    vstarts = [sum(VP[:j]) for j in range(ns)]
    nb = U // CB
    upb = sk // U
    n_units = n_kv * upb
    nk = AK + 1
    nv = AV + 1
    hw = 2 * dh
    f32 = jnp.float32
    bf16 = jnp.bfloat16
    nt_dims = (((1,), (1,)), ((), ()))

    def k_copy(u, j):
        slot = u % nk
        return pltpu.make_async_copy(
            k_hbm.at[pl.ds(u * U + kstarts[j], KP[j])],
            kbuf.at[slot, pl.ds(kstarts[j], KP[j])], ksem.at[slot])

    def v_copy(u, j):
        slot = u % nv
        return pltpu.make_async_copy(
            v_hbm.at[pl.ds(u * U + vstarts[j], VP[j])],
            vbuf.at[slot, pl.ds(vstarts[j], VP[j])], vsem.at[slot, j])

    def wait_all(buf, sem):
        pltpu.make_async_copy(buf, buf, sem).wait()

    def k_wait(u):
        wait_all(kbuf.at[u % nk], ksem.at[u % nk])

    n_rg = d_model // 8
    n_w16 = d_model // 16
    ffn_per_head = (3 * n_rg) // n_kv
    n_extra = 2 * n_w16 + ffn_per_head
    assert ffn_per_head * n_kv == 3 * n_rg and n_extra <= upb - upb // 4 and n_w16 <= upb // 2

    def head_piece(src, dst, sem, h, i):
        col = pl.multiple_of(h * hw, hw)
        row = pl.multiple_of(i * 16, 16)
        return pltpu.make_async_copy(src.at[pl.ds(row, 16), pl.ds(col, hw)],
                                     dst.at[h, pl.ds(row, 16)], sem.at[h])

    def ffn_piece(src, dst, sem, i):
        row = pl.multiple_of(i * 8, 8)
        return pltpu.make_async_copy(src.at[pl.ds(row, 8)], dst.at[pl.ds(row, 8)], sem)

    def issue_weight_piece(h, r):
        @pl.when(r < n_extra)
        def _():
            @pl.when(jnp.logical_and(r < n_w16, h < n_kv - 1))
            def _():
                head_piece(wq_hbm, wqbuf, wqsem, h + 1, r).start(priority=HI)

            @pl.when(jnp.logical_and(r >= n_w16, r < 2 * n_w16))
            def _():
                head_piece(wot_hbm, wobuf, wosem, h, r - n_w16).start(priority=HI)

            f = h * ffn_per_head + r - 2 * n_w16

            @pl.when(r >= 2 * n_w16)
            def _():
                @pl.when(f < n_rg)
                def _():
                    ffn_piece(wg_hbm, wgbuf, msem.at[2], f).start(priority=HI)

                @pl.when(jnp.logical_and(f >= n_rg, f < 2 * n_rg))
                def _():
                    ffn_piece(wu_hbm, wubuf, msem.at[3], f - n_rg).start(priority=HI)

                @pl.when(f >= 2 * n_rg)
                def _():
                    ffn_piece(wdt_hbm, wdbuf, msem.at[4], f - 2 * n_rg).start(priority=HI)

    x_copy = pltpu.make_async_copy(x_hbm, xbuf, msem.at[0])
    wr_copy = pltpu.make_async_copy(wr_hbm, wrbuf, msem.at[1])
    wq0_copy = pltpu.make_async_copy(wq_hbm.at[:, pl.ds(0, hw)], wqbuf.at[0], wqsem.at[0])
    out_copy = pltpu.make_async_copy(obuf, o_hbm, msem.at[5])

    x_copy.start(priority=HI)
    wr_copy.start(priority=HI)
    wq0_copy.start(priority=HI)

    def k_init(u, c):
        for j in range(nkp):
            k_copy(u, j).start(priority=HI)
        return c

    def v_init(u, c):
        for j in range(ns):
            v_copy(u, j).start(priority=LO)
        return c

    jax.lax.fori_loop(0, AK + 1, k_init, 0)
    jax.lax.fori_loop(0, AV, v_init, 0)

    x_copy.wait()
    x = xbuf[0].astype(f32)
    mu = jnp.mean(x, axis=1, keepdims=True)
    xc = x - mu
    var = jnp.mean(xc * xc, axis=1, keepdims=True)
    xn = (xc / jnp.sqrt(var + 1e-5)).astype(bf16)
    xn_scr[...] = jnp.broadcast_to(xn, (8, d_model))

    row = jax.lax.broadcasted_iota(jnp.int32, (8, dh), 0)
    top = row < 4

    def make_q(h):
        qf = jnp.dot(xn_scr[...], wqbuf[h], preferred_element_type=f32)
        qh = jnp.where(top, qf[:, :dh], qf[:, dh:]).astype(bf16)
        q_scr[h] = (qh.astype(f32) * (dh ** -0.5)).astype(bf16)

    wq0_copy.wait()
    make_q(0)
    out_scr[...] = jnp.zeros(out_scr.shape, f32)

    def qk(u):
        q = q_scr[u // upb]
        return [jax.lax.dot_general(q, kbuf[u % nk, pl.ds(b * CB, CB), :], nt_dims,
                                    preferred_element_type=f32) for b in range(nb)]

    def softmax(u, s_parts, m, l):
        first = (u % upb) == 0
        m_prev = jnp.where(first, NEG, m)
        l_prev = jnp.where(first, 0.0, l)
        s = jnp.concatenate(s_parts, axis=1)
        m_new = jnp.maximum(m_prev, jnp.max(s, axis=1, keepdims=True))
        p = jnp.exp(s - m_new)
        alpha = jnp.exp(m_prev - m_new)
        ps = p[:, 0:128]
        for c in range(1, U // 128):
            ps = ps + p[:, c * 128:(c + 1) * 128]
        return p.astype(bf16), alpha, m_new, alpha * l_prev + ps

    def pv(u, p):
        res = None
        for b in range(nb):
            t = jnp.dot(p[:, b * CB:(b + 1) * CB], vbuf[u % nv, pl.ds(b * CB, CB), :],
                        preferred_element_type=f32)
            res = t if res is None else res + t
        return res

    def project(h, o):
        lhs = jnp.concatenate([jnp.where(row == 0, o, 0.0), jnp.where(row == 4, o, 0.0)],
                              axis=1).astype(bf16)
        return jax.lax.dot_general(lhs, wobuf[h], nt_dims, preferred_element_type=f32)

    def ffn():
        wait_all(wgbuf, msem.at[2])
        wait_all(wubuf, msem.at[3])
        wait_all(wdbuf, msem.at[4])
        wr_copy.wait()
        xb = xn_scr[...]
        g = jnp.dot(xb, wgbuf[...], preferred_element_type=f32).astype(bf16).astype(f32)
        up = jnp.dot(xb, wubuf[...], preferred_element_type=f32).astype(bf16).astype(f32)
        g = (g * jax.nn.sigmoid(g)).astype(bf16)
        hid = (g.astype(f32) * up).astype(bf16)
        y = jax.lax.dot_general(hid, wdbuf[...], nt_dims, preferred_element_type=f32)
        xf = xb.astype(f32)
        wr = wrbuf[...].astype(f32).reshape(1, d_model)
        rs = jax.nn.sigmoid(jnp.sum(xf * wr, axis=1, keepdims=True))
        rows = jax.lax.broadcasted_iota(jnp.int32, (8, d_model), 0)
        base = xbuf[0].astype(f32) + xf + xf * 0.0 + y * rs
        out_scr[...] += jnp.where(rows == 0, base, 0.0)

    k_wait(0)
    p0, a0, m0, l0 = softmax(0, qk(0), jnp.full((8, 1), NEG, f32), jnp.zeros((8, 128), f32))
    acc0 = jnp.zeros((8, dh), f32)

    def body(u, carry, issue_k, issue_v, main):
        p, alpha, m, l, acc = carry
        h = u // upb
        r = u % upb
        for j in range(ns):
            v_copy(u, j).wait()
            if issue_k:
                for jk in range(nkp):
                    if KEV[jk] == j:
                        k_copy(u + 1 + AK, jk).start(priority=HI)
            if issue_v:
                v_copy(u + AV, j).start(priority=LO)
            if main and j == XEV:
                issue_weight_piece(h, r)
            if j == 0:
                k_wait(u + 1)
                s_parts = qk(u + 1)
            if j == 1:
                nxt = softmax(u + 1, s_parts, m, l)
        acc = alpha * acc + pv(u, p)

        if main:
            @pl.when(jnp.logical_and(r == upb // 2, h < n_kv - 1))
            def _():
                wait_all(wqbuf.at[h + 1], wqsem.at[h + 1])
                make_q(h + 1)

            @pl.when(u == n_units - upb // 4)
            def _():
                ffn()

            @pl.when(r == upb - 1)
            def _():
                o = acc / jnp.sum(l, axis=1, keepdims=True)
                wait_all(wobuf.at[h], wosem.at[h])
                out_scr[...] += project(h, o)
        return nxt + (acc,)

    carry = (p0, a0, m0, l0, acc0)
    marks = sorted({n_units - AV, n_units - AK - 1, n_units - 1})
    assert marks[0] > n_units - upb // 4
    lo = 0
    for hi in marks:
        flags = dict(issue_k=hi <= n_units - AK - 1, issue_v=hi <= n_units - AV, main=lo == 0)
        carry = jax.lax.fori_loop(lo, hi, functools.partial(
            lambda u, c, fl: body(u, c, **fl), fl=flags), carry)
        lo = hi

    p, alpha, m, l, acc = carry
    u = n_units - 1
    wait_all(wobuf.at[n_kv - 1], wosem.at[n_kv - 1])
    rinv = 1.0 / jnp.sum(l, axis=1, keepdims=True)
    acc = alpha * acc
    for j in range(ns):
        v_copy(u, j).wait()
    acc = acc + pv(u, p)
    tot = out_scr[...] + project(n_kv - 1, acc * rinv)
    obuf[0] = jnp.sum(tot, axis=0, keepdims=True).astype(obuf.dtype)
    out_copy.start()
    out_copy.wait()


@jax.jit
def pallas_parallel_sum__gqa_block_cached__moe_arch_mod__decode_kernel(
    A_x: jax.Array,
    A_k_cache: jax.Array,
    A_v_cache: jax.Array,
    A_wq: jax.Array,
    A_wo: jax.Array,
    B_x: jax.Array,
    B_w_r: jax.Array,
    B_w_gate: jax.Array,
    B_w_up: jax.Array,
    B_w_down: jax.Array,
):
    del B_x
    _, n_kv, sk, dh = A_k_cache.shape
    d_model = A_x.shape[-1]
    assert A_wq.shape[1] == 2 * n_kv * dh and A_x.shape == (1, 1, d_model)
    ffn = B_w_gate.shape[1]
    hw = 2 * dh
    ns = len(VP)
    bf16 = jnp.bfloat16

    k2 = A_k_cache.reshape(n_kv * sk, dh)
    v2 = A_v_cache.reshape(n_kv * sk, dh)
    wot = A_wo.T
    wdt = B_w_down.T

    kernel = functools.partial(_kernel, n_kv=n_kv, sk=sk, dh=dh, d_model=d_model)
    return pl.pallas_call(
        kernel,
        out_shape=jax.ShapeDtypeStruct((1, 1, d_model), A_x.dtype),
        in_specs=[pl.BlockSpec(memory_space=pl.ANY)] * 9,
        out_specs=pl.BlockSpec(memory_space=pl.ANY),
        scratch_shapes=[
            pltpu.VMEM((1, 1, d_model), bf16),
            pltpu.VMEM((d_model,), bf16),
            pltpu.VMEM((1, 1, d_model), bf16),
            pltpu.VMEM((AK + 1, U, dh), bf16),
            pltpu.VMEM((AV + 1, U, dh), bf16),
            pltpu.VMEM((n_kv, d_model, hw), bf16),
            pltpu.VMEM((n_kv, d_model, hw), bf16),
            pltpu.VMEM((d_model, ffn), bf16),
            pltpu.VMEM((d_model, ffn), bf16),
            pltpu.VMEM((d_model, ffn), bf16),
            pltpu.VMEM((8, d_model), bf16),
            pltpu.VMEM((n_kv, 8, dh), bf16),
            pltpu.VMEM((8, d_model), jnp.float32),
            pltpu.SemaphoreType.DMA((AK + 1,)),
            pltpu.SemaphoreType.DMA((AV + 1, ns)),
            pltpu.SemaphoreType.DMA((n_kv,)),
            pltpu.SemaphoreType.DMA((n_kv,)),
            pltpu.SemaphoreType.DMA((6,)),
        ],
        compiler_params=pltpu.CompilerParams(vmem_limit_bytes=64 * 1024 * 1024,
                                             disable_bounds_checks=True,
                                             disable_semaphore_checks=True),
    )(A_x, k2, v2, A_wq, wot, B_w_r, B_w_gate, B_w_up, wdt)
```

```python
import functools

import jax
import jax.numpy as jnp
import jax.experimental.pallas as pl
import jax.experimental.pallas.tpu as pltpu


HI = 0
LO = 1

U = 512
KP = (56, 128, 128, 120, 80)
KEV = (0, 1, 3, 4, 5)
VP = (48, 120, 16, 120, 120, 88)
AK = 3
AV = 7
XEV = 1
CB = 256
NFIN = 3
NEG = -1e30


def _kernel(x_hbm, k_hbm, v_hbm, wq_hbm, wot_hbm, wr_hbm, wg_hbm, wu_hbm, wdt_hbm,
            o_hbm,
            xbuf, wrbuf, obuf, kbuf, vbuf, wqbuf, wobuf, wgbuf, wubuf, wdbuf,
            xn_scr, q_scr, out_scr,
            ksem, vsem, wqsem, wosem, msem,
            *, n_kv, sk, dh, d_model):
    ns = len(VP)
    nkp = len(KP)
    assert len(KEV) == nkp and max(KEV) < ns and sum(KP) == U and sum(VP) == U
    kstarts = [sum(KP[:j]) for j in range(nkp)]
    vstarts = [sum(VP[:j]) for j in range(ns)]
    nb = U // CB
    upb = sk // U
    n_units = n_kv * upb
    nk = AK + 1
    nv = AV + 1
    hw = 2 * dh
    f32 = jnp.float32
    bf16 = jnp.bfloat16
    nt_dims = (((1,), (1,)), ((), ()))

    def k_copy(u, j):
        slot = u % nk
        return pltpu.make_async_copy(
            k_hbm.at[pl.ds(u * U + kstarts[j], KP[j])],
            kbuf.at[slot, pl.ds(kstarts[j], KP[j])], ksem.at[slot])

    def v_copy(u, j):
        slot = u % nv
        return pltpu.make_async_copy(
            v_hbm.at[pl.ds(u * U + vstarts[j], VP[j])],
            vbuf.at[slot, pl.ds(vstarts[j], VP[j])], vsem.at[slot, j])

    def wait_all(buf, sem):
        pltpu.make_async_copy(buf, buf, sem).wait()

    def k_wait(u):
        wait_all(kbuf.at[u % nk], ksem.at[u % nk])

    n_rg = d_model // 8
    n_w16 = d_model // 16
    ffn_per_head = (3 * n_rg) // n_kv
    n_extra = 2 * n_w16 + ffn_per_head
    assert ffn_per_head * n_kv == 3 * n_rg and n_extra <= upb - upb // 4 and n_w16 <= upb // 2

    def head_piece(src, dst, sem, h, i):
        col = pl.multiple_of(h * hw, hw)
        row = pl.multiple_of(i * 16, 16)
        return pltpu.make_async_copy(src.at[pl.ds(row, 16), pl.ds(col, hw)],
                                     dst.at[h, pl.ds(row, 16)], sem.at[h])

    def ffn_piece(src, dst, sem, i):
        row = pl.multiple_of(i * 8, 8)
        return pltpu.make_async_copy(src.at[pl.ds(row, 8)], dst.at[pl.ds(row, 8)], sem)

    def issue_weight_piece(h, r):
        @pl.when(r < n_extra)
        def _():
            @pl.when(jnp.logical_and(r < n_w16, h < n_kv - 1))
            def _():
                head_piece(wq_hbm, wqbuf, wqsem, h + 1, r).start(priority=HI)

            @pl.when(jnp.logical_and(r >= n_w16, r < 2 * n_w16))
            def _():
                head_piece(wot_hbm, wobuf, wosem, h, r - n_w16).start(priority=HI)

            f = h * ffn_per_head + r - 2 * n_w16

            @pl.when(r >= 2 * n_w16)
            def _():
                @pl.when(f < n_rg)
                def _():
                    ffn_piece(wg_hbm, wgbuf, msem.at[2], f).start(priority=HI)

                @pl.when(jnp.logical_and(f >= n_rg, f < 2 * n_rg))
                def _():
                    ffn_piece(wu_hbm, wubuf, msem.at[3], f - n_rg).start(priority=HI)

                @pl.when(f >= 2 * n_rg)
                def _():
                    ffn_piece(wdt_hbm, wdbuf, msem.at[4], f - 2 * n_rg).start(priority=HI)

    x_copy = pltpu.make_async_copy(x_hbm, xbuf, msem.at[0])
    wr_copy = pltpu.make_async_copy(wr_hbm, wrbuf, msem.at[1])
    wq0_copy = pltpu.make_async_copy(wq_hbm.at[:, pl.ds(0, hw)], wqbuf.at[0], wqsem.at[0])
    out_copy = pltpu.make_async_copy(obuf, o_hbm, msem.at[5])

    x_copy.start(priority=HI)
    wr_copy.start(priority=HI)
    wq0_copy.start(priority=HI)

    def k_init(u, c):
        for j in range(nkp):
            k_copy(u, j).start(priority=HI)
        return c

    def v_init(u, c):
        for j in range(ns):
            v_copy(u, j).start(priority=LO)
        return c

    jax.lax.fori_loop(0, AK + 1, k_init, 0)
    jax.lax.fori_loop(0, AV, v_init, 0)

    x_copy.wait()
    x = xbuf[0].astype(f32)
    mu = jnp.mean(x, axis=1, keepdims=True)
    xc = x - mu
    var = jnp.mean(xc * xc, axis=1, keepdims=True)
    xn = (xc / jnp.sqrt(var + 1e-5)).astype(bf16)
    xn_scr[...] = jnp.broadcast_to(xn, (8, d_model))

    row = jax.lax.broadcasted_iota(jnp.int32, (8, dh), 0)
    top = row < 4

    def make_q(h):
        qf = jnp.dot(xn_scr[...], wqbuf[h], preferred_element_type=f32)
        qh = jnp.where(top, qf[:, :dh], qf[:, dh:]).astype(bf16)
        q_scr[h] = (qh.astype(f32) * (dh ** -0.5)).astype(bf16)

    wq0_copy.wait()
    make_q(0)
    out_scr[...] = jnp.zeros(out_scr.shape, f32)

    def qk(u):
        q = q_scr[u // upb]
        return [jax.lax.dot_general(q, kbuf[u % nk, pl.ds(b * CB, CB), :], nt_dims,
                                    preferred_element_type=f32) for b in range(nb)]

    def softmax(first, s_parts, m, l):
        if first is not None:
            m = jnp.where(first, NEG, m)
            l = jnp.where(first, 0.0, l)
        s = jnp.concatenate(s_parts, axis=1)
        m_new = jnp.maximum(m, jnp.max(s, axis=1, keepdims=True))
        p = jnp.exp(s - m_new)
        alpha = jnp.exp(m - m_new)
        ps = p[:, 0:128]
        for c in range(1, s.shape[1] // 128):
            ps = ps + p[:, c * 128:(c + 1) * 128]
        return p.astype(bf16), alpha, m_new, alpha * l + ps

    def pv(u, p):
        res = None
        for b in range(nb):
            t = jnp.dot(p[:, b * CB:(b + 1) * CB], vbuf[u % nv, pl.ds(b * CB, CB), :],
                        preferred_element_type=f32)
            res = t if res is None else res + t
        return res

    def project(h, o):
        lhs = jnp.concatenate([jnp.where(row == 0, o, 0.0), jnp.where(row == 4, o, 0.0)],
                              axis=1).astype(bf16)
        return jax.lax.dot_general(lhs, wobuf[h], nt_dims, preferred_element_type=f32)

    def ffn():
        wait_all(wgbuf, msem.at[2])
        wait_all(wubuf, msem.at[3])
        wait_all(wdbuf, msem.at[4])
        wr_copy.wait()
        xb = xn_scr[...]
        g = jnp.dot(xb, wgbuf[...], preferred_element_type=f32).astype(bf16).astype(f32)
        up = jnp.dot(xb, wubuf[...], preferred_element_type=f32).astype(bf16).astype(f32)
        g = (g * jax.nn.sigmoid(g)).astype(bf16)
        hid = (g.astype(f32) * up).astype(bf16)
        y = jax.lax.dot_general(hid, wdbuf[...], nt_dims, preferred_element_type=f32)
        xf = xb.astype(f32)
        wr = wrbuf[...].astype(f32).reshape(1, d_model)
        rs = jax.nn.sigmoid(jnp.sum(xf * wr, axis=1, keepdims=True))
        rows = jax.lax.broadcasted_iota(jnp.int32, (8, d_model), 0)
        base = xbuf[0].astype(f32) + xf + xf * 0.0 + y * rs
        out_scr[...] += jnp.where(rows == 0, base, 0.0)

    k_wait(0)
    p0, a0, m0, l0 = softmax(None, qk(0), jnp.full((8, 1), NEG, f32), jnp.zeros((8, 128), f32))
    acc0 = jnp.zeros((8, dh), f32)

    def body(u, carry):
        p, alpha, m, l, acc = carry
        h = u // upb
        r = u % upb
        issue_k = u + 1 + AK < n_units
        issue_v = u + AV < n_units
        for j in range(ns):
            v_copy(u, j).wait()
            for jk in range(nkp):
                if KEV[jk] == j:
                    @pl.when(issue_k)
                    def _():
                        k_copy(u + 1 + AK, jk).start(priority=HI)

            @pl.when(issue_v)
            def _():
                v_copy(u + AV, j).start(priority=LO)

            if j == XEV:
                issue_weight_piece(h, r)
            if j == 0:
                k_wait(u + 1)
                s_parts = qk(u + 1)
            if j == 1:
                nxt = softmax((u + 1) % upb == 0, s_parts, m, l)
        acc = alpha * acc + pv(u, p)

        @pl.when(jnp.logical_and(r == upb // 2, h < n_kv - 1))
        def _():
            wait_all(wqbuf.at[h + 1], wqsem.at[h + 1])
            make_q(h + 1)

        @pl.when(u == n_units - upb // 4)
        def _():
            ffn()

        @pl.when(r == upb - 1)
        def _():
            o = acc / jnp.sum(l, axis=1, keepdims=True)
            wait_all(wobuf.at[h], wosem.at[h])
            out_scr[...] += project(h, o)
        return nxt + (acc,)

    assert 1 <= NFIN <= upb // 4
    carry = jax.lax.fori_loop(0, n_units - NFIN, body, (p0, a0, m0, l0, acc0))

    p, alpha, m, l, acc = carry
    u0 = n_units - NFIN
    if NFIN > 1:
        s_parts = []
        for u in range(u0 + 1, n_units):
            k_wait(u)
            s_parts += qk(u)
        p2, alpha2, _, l = softmax(None, s_parts, m, l)
    rinv = 1.0 / jnp.sum(l, axis=1, keepdims=True)
    wait_all(wobuf.at[n_kv - 1], wosem.at[n_kv - 1])
    acc = alpha * acc
    for j in range(ns):
        v_copy(u0, j).wait()
    acc = acc + pv(u0, p)
    if NFIN > 1:
        acc = alpha2 * acc
    for i, u in enumerate(range(u0 + 1, n_units)):
        for j in range(ns):
            v_copy(u, j).wait()
        acc = acc + pv(u, p2[:, i * U:(i + 1) * U])
    tot = out_scr[...] + project(n_kv - 1, acc * rinv)
    obuf[0] = jnp.sum(tot, axis=0, keepdims=True).astype(obuf.dtype)
    out_copy.start()
    out_copy.wait()


@jax.jit
def pallas_parallel_sum__gqa_block_cached__moe_arch_mod__decode_kernel(
    A_x: jax.Array,
    A_k_cache: jax.Array,
    A_v_cache: jax.Array,
    A_wq: jax.Array,
    A_wo: jax.Array,
    B_x: jax.Array,
    B_w_r: jax.Array,
    B_w_gate: jax.Array,
    B_w_up: jax.Array,
    B_w_down: jax.Array,
):
    del B_x
    _, n_kv, sk, dh = A_k_cache.shape
    d_model = A_x.shape[-1]
    assert A_wq.shape[1] == 2 * n_kv * dh and A_x.shape == (1, 1, d_model)
    ffn = B_w_gate.shape[1]
    hw = 2 * dh
    ns = len(VP)
    bf16 = jnp.bfloat16

    k2 = A_k_cache.reshape(n_kv * sk, dh)
    v2 = A_v_cache.reshape(n_kv * sk, dh)
    wot = A_wo.T
    wdt = B_w_down.T

    kernel = functools.partial(_kernel, n_kv=n_kv, sk=sk, dh=dh, d_model=d_model)
    return pl.pallas_call(
        kernel,
        out_shape=jax.ShapeDtypeStruct((1, 1, d_model), A_x.dtype),
        in_specs=[pl.BlockSpec(memory_space=pl.ANY)] * 9,
        out_specs=pl.BlockSpec(memory_space=pl.ANY),
        scratch_shapes=[
            pltpu.VMEM((1, 1, d_model), bf16),
            pltpu.VMEM((d_model,), bf16),
            pltpu.VMEM((1, 1, d_model), bf16),
            pltpu.VMEM((AK + 1, U, dh), bf16),
            pltpu.VMEM((AV + 1, U, dh), bf16),
            pltpu.VMEM((n_kv, d_model, hw), bf16),
            pltpu.VMEM((n_kv, d_model, hw), bf16),
            pltpu.VMEM((d_model, ffn), bf16),
            pltpu.VMEM((d_model, ffn), bf16),
            pltpu.VMEM((d_model, ffn), bf16),
            pltpu.VMEM((8, d_model), bf16),
            pltpu.VMEM((n_kv, 8, dh), bf16),
            pltpu.VMEM((8, d_model), jnp.float32),
            pltpu.SemaphoreType.DMA((AK + 1,)),
            pltpu.SemaphoreType.DMA((AV + 1, ns)),
            pltpu.SemaphoreType.DMA((n_kv,)),
            pltpu.SemaphoreType.DMA((n_kv,)),
            pltpu.SemaphoreType.DMA((6,)),
        ],
        compiler_params=pltpu.CompilerParams(vmem_limit_bytes=64 * 1024 * 1024,
                                             disable_bounds_checks=True,
                                             disable_semaphore_checks=True),
    )(A_x, k2, v2, A_wq, wot, B_w_r, B_w_gate, B_w_up, wdt)
```

```python
import functools

import jax
import jax.numpy as jnp
import jax.experimental.pallas as pl
import jax.experimental.pallas.tpu as pltpu


HI = 0
LO = 1

U = 512
KP = (56, 128, 128, 120, 80)
KEV = (0, 1, 3, 4, 5)
VP = (48, 120, 24, 112, 120, 88)
AK = 3
AV = 7
XEV = 0
QK_EV = 0
SM_EV = 1
CB = 256
NFIN = 3
NEG = -1e30


def _kernel(x_hbm, k_hbm, v_hbm, wq_hbm, wot_hbm, wr_hbm, wg_hbm, wu_hbm, wdt_hbm,
            o_hbm,
            xbuf, wrbuf, obuf, kbuf, vbuf, wqbuf, wobuf, wgbuf, wubuf, wdbuf,
            xn_scr, q_scr, out_scr,
            ksem, vsem, wqsem, wosem, msem,
            *, n_kv, sk, dh, d_model):
    ns = len(VP)
    nkp = len(KP)
    assert len(KEV) == nkp and max(KEV) < ns and sum(KP) == U and sum(VP) == U
    kstarts = [sum(KP[:j]) for j in range(nkp)]
    vstarts = [sum(VP[:j]) for j in range(ns)]
    nb = U // CB
    upb = sk // U
    n_units = n_kv * upb
    nk = AK + 1
    nv = AV + 1
    hw = 2 * dh
    f32 = jnp.float32
    bf16 = jnp.bfloat16
    nt_dims = (((1,), (1,)), ((), ()))

    def k_copy(u, j):
        slot = u % nk
        return pltpu.make_async_copy(
            k_hbm.at[pl.ds(u * U + kstarts[j], KP[j])],
            kbuf.at[slot, pl.ds(kstarts[j], KP[j])], ksem.at[slot])

    def v_copy(u, j):
        slot = u % nv
        return pltpu.make_async_copy(
            v_hbm.at[pl.ds(u * U + vstarts[j], VP[j])],
            vbuf.at[slot, pl.ds(vstarts[j], VP[j])], vsem.at[slot, j])

    def wait_all(buf, sem):
        pltpu.make_async_copy(buf, buf, sem).wait()

    def k_wait(u):
        wait_all(kbuf.at[u % nk], ksem.at[u % nk])

    n_rg = d_model // 8
    n_w16 = d_model // 16
    ffn_per_head = (3 * n_rg) // n_kv
    n_extra = 2 * n_w16 + ffn_per_head
    assert ffn_per_head * n_kv == 3 * n_rg and n_extra <= upb - upb // 4 and n_w16 <= upb // 2

    def head_piece(src, dst, sem, h, i):
        col = pl.multiple_of(h * hw, hw)
        row = pl.multiple_of(i * 16, 16)
        return pltpu.make_async_copy(src.at[pl.ds(row, 16), pl.ds(col, hw)],
                                     dst.at[h, pl.ds(row, 16)], sem.at[h])

    def ffn_piece(src, dst, sem, i):
        row = pl.multiple_of(i * 8, 8)
        return pltpu.make_async_copy(src.at[pl.ds(row, 8)], dst.at[pl.ds(row, 8)], sem)

    def issue_weight_piece(h, r):
        @pl.when(r < n_extra)
        def _():
            @pl.when(jnp.logical_and(r < n_w16, h < n_kv - 1))
            def _():
                head_piece(wq_hbm, wqbuf, wqsem, h + 1, r).start(priority=HI)

            @pl.when(jnp.logical_and(r >= n_w16, r < 2 * n_w16))
            def _():
                head_piece(wot_hbm, wobuf, wosem, h, r - n_w16).start(priority=HI)

            f = h * ffn_per_head + r - 2 * n_w16

            @pl.when(r >= 2 * n_w16)
            def _():
                @pl.when(f < n_rg)
                def _():
                    ffn_piece(wg_hbm, wgbuf, msem.at[2], f).start(priority=HI)

                @pl.when(jnp.logical_and(f >= n_rg, f < 2 * n_rg))
                def _():
                    ffn_piece(wu_hbm, wubuf, msem.at[3], f - n_rg).start(priority=HI)

                @pl.when(f >= 2 * n_rg)
                def _():
                    ffn_piece(wdt_hbm, wdbuf, msem.at[4], f - 2 * n_rg).start(priority=HI)

    x_copy = pltpu.make_async_copy(x_hbm, xbuf, msem.at[0])
    wr_copy = pltpu.make_async_copy(wr_hbm, wrbuf, msem.at[1])
    wq0_copy = pltpu.make_async_copy(wq_hbm.at[:, pl.ds(0, hw)], wqbuf.at[0], wqsem.at[0])
    out_copy = pltpu.make_async_copy(obuf, o_hbm, msem.at[5])

    x_copy.start(priority=HI)
    wr_copy.start(priority=HI)
    wq0_copy.start(priority=HI)

    def k_init(u, c):
        for j in range(nkp):
            k_copy(u, j).start(priority=HI)
        return c

    def v_init(u, c):
        for j in range(ns):
            v_copy(u, j).start(priority=LO)
        return c

    jax.lax.fori_loop(0, AK + 1, k_init, 0)
    jax.lax.fori_loop(0, AV, v_init, 0)

    x_copy.wait()
    x = xbuf[0].astype(f32)
    mu = jnp.mean(x, axis=1, keepdims=True)
    xc = x - mu
    var = jnp.mean(xc * xc, axis=1, keepdims=True)
    xn = (xc / jnp.sqrt(var + 1e-5)).astype(bf16)
    xn_scr[...] = jnp.broadcast_to(xn, (8, d_model))

    row = jax.lax.broadcasted_iota(jnp.int32, (8, dh), 0)
    top = row < 4

    def make_q(h):
        qf = jnp.dot(xn_scr[...], wqbuf[h], preferred_element_type=f32)
        qh = jnp.where(top, qf[:, :dh], qf[:, dh:]).astype(bf16)
        q_scr[h] = (qh.astype(f32) * (dh ** -0.5)).astype(bf16)

    wq0_copy.wait()
    make_q(0)
    out_scr[...] = jnp.zeros(out_scr.shape, f32)

    def qk(u):
        q = q_scr[u // upb]
        return [jax.lax.dot_general(q, kbuf[u % nk, pl.ds(b * CB, CB), :], nt_dims,
                                    preferred_element_type=f32) for b in range(nb)]

    def softmax(first, s_parts, m, l):
        if first is not None:
            m = jnp.where(first, NEG, m)
            l = jnp.where(first, 0.0, l)
        s = jnp.concatenate(s_parts, axis=1)
        m_new = jnp.maximum(m, jnp.max(s, axis=1, keepdims=True))
        p = jnp.exp(s - m_new)
        alpha = jnp.exp(m - m_new)
        ps = p[:, 0:128]
        for c in range(1, s.shape[1] // 128):
            ps = ps + p[:, c * 128:(c + 1) * 128]
        return p.astype(bf16), alpha, m_new, alpha * l + ps

    def pv(u, p):
        res = None
        for b in range(nb):
            t = jnp.dot(p[:, b * CB:(b + 1) * CB], vbuf[u % nv, pl.ds(b * CB, CB), :],
                        preferred_element_type=f32)
            res = t if res is None else res + t
        return res

    def project(h, o):
        lhs = jnp.concatenate([jnp.where(row == 0, o, 0.0), jnp.where(row == 4, o, 0.0)],
                              axis=1).astype(bf16)
        return jax.lax.dot_general(lhs, wobuf[h], nt_dims, preferred_element_type=f32)

    def ffn():
        wait_all(wgbuf, msem.at[2])
        wait_all(wubuf, msem.at[3])
        wait_all(wdbuf, msem.at[4])
        wr_copy.wait()
        xb = xn_scr[...]
        g = jnp.dot(xb, wgbuf[...], preferred_element_type=f32).astype(bf16).astype(f32)
        up = jnp.dot(xb, wubuf[...], preferred_element_type=f32).astype(bf16).astype(f32)
        g = (g * jax.nn.sigmoid(g)).astype(bf16)
        hid = (g.astype(f32) * up).astype(bf16)
        y = jax.lax.dot_general(hid, wdbuf[...], nt_dims, preferred_element_type=f32)
        xf = xb.astype(f32)
        wr = wrbuf[...].astype(f32).reshape(1, d_model)
        rs = jax.nn.sigmoid(jnp.sum(xf * wr, axis=1, keepdims=True))
        rows = jax.lax.broadcasted_iota(jnp.int32, (8, d_model), 0)
        base = xbuf[0].astype(f32) + xf + xf * 0.0 + y * rs
        out_scr[...] += jnp.where(rows == 0, base, 0.0)

    k_wait(0)
    p0, a0, m0, l0 = softmax(None, qk(0), jnp.full((8, 1), NEG, f32), jnp.zeros((8, 128), f32))
    acc0 = jnp.zeros((8, dh), f32)

    def body(u, carry):
        p, alpha, m, l, acc = carry
        h = u // upb
        r = u % upb
        issue_k = u + 1 + AK < n_units
        issue_v = u + AV < n_units
        for j in range(ns):
            v_copy(u, j).wait()
            for jk in range(nkp):
                if KEV[jk] == j:
                    @pl.when(issue_k)
                    def _():
                        k_copy(u + 1 + AK, jk).start(priority=HI)

            @pl.when(issue_v)
            def _():
                v_copy(u + AV, j).start(priority=LO)

            if j == XEV:
                issue_weight_piece(h, r)
            if j == QK_EV:
                k_wait(u + 1)
                s_parts = qk(u + 1)
            if j == SM_EV:
                nxt = softmax((u + 1) % upb == 0, s_parts, m, l)
        acc = alpha * acc + pv(u, p)

        @pl.when(jnp.logical_and(r == upb // 2, h < n_kv - 1))
        def _():
            wait_all(wqbuf.at[h + 1], wqsem.at[h + 1])
            make_q(h + 1)

        @pl.when(u == n_units - upb // 4)
        def _():
            ffn()

        @pl.when(r == upb - 1)
        def _():
            o = acc / jnp.sum(l, axis=1, keepdims=True)
            wait_all(wobuf.at[h], wosem.at[h])
            out_scr[...] += project(h, o)
        return nxt + (acc,)

    assert 1 <= NFIN <= upb // 4
    carry = jax.lax.fori_loop(0, n_units - NFIN, body, (p0, a0, m0, l0, acc0))

    p, alpha, m, l, acc = carry
    u0 = n_units - NFIN
    if NFIN > 1:
        s_parts = []
        for u in range(u0 + 1, n_units):
            k_wait(u)
            s_parts += qk(u)
        p2, alpha2, _, l = softmax(None, s_parts, m, l)
    rinv = 1.0 / jnp.sum(l, axis=1, keepdims=True)
    wait_all(wobuf.at[n_kv - 1], wosem.at[n_kv - 1])
    acc = alpha * acc
    for j in range(ns):
        v_copy(u0, j).wait()
    acc = acc + pv(u0, p)
    if NFIN > 1:
        acc = alpha2 * acc
    for i, u in enumerate(range(u0 + 1, n_units)):
        for j in range(ns):
            v_copy(u, j).wait()
        acc = acc + pv(u, p2[:, i * U:(i + 1) * U])
    tot = out_scr[...] + project(n_kv - 1, acc * rinv)
    obuf[0] = jnp.sum(tot, axis=0, keepdims=True).astype(obuf.dtype)
    out_copy.start()
    out_copy.wait()


@jax.jit
def pallas_parallel_sum__gqa_block_cached__moe_arch_mod__decode_kernel(
    A_x: jax.Array,
    A_k_cache: jax.Array,
    A_v_cache: jax.Array,
    A_wq: jax.Array,
    A_wo: jax.Array,
    B_x: jax.Array,
    B_w_r: jax.Array,
    B_w_gate: jax.Array,
    B_w_up: jax.Array,
    B_w_down: jax.Array,
):
    del B_x
    _, n_kv, sk, dh = A_k_cache.shape
    d_model = A_x.shape[-1]
    assert A_wq.shape[1] == 2 * n_kv * dh and A_x.shape == (1, 1, d_model)
    ffn = B_w_gate.shape[1]
    hw = 2 * dh
    ns = len(VP)
    bf16 = jnp.bfloat16

    k2 = A_k_cache.reshape(n_kv * sk, dh)
    v2 = A_v_cache.reshape(n_kv * sk, dh)
    wot = A_wo.T
    wdt = B_w_down.T

    kernel = functools.partial(_kernel, n_kv=n_kv, sk=sk, dh=dh, d_model=d_model)
    return pl.pallas_call(
        kernel,
        out_shape=jax.ShapeDtypeStruct((1, 1, d_model), A_x.dtype),
        in_specs=[pl.BlockSpec(memory_space=pl.ANY)] * 9,
        out_specs=pl.BlockSpec(memory_space=pl.ANY),
        scratch_shapes=[
            pltpu.VMEM((1, 1, d_model), bf16),
            pltpu.VMEM((d_model,), bf16),
            pltpu.VMEM((1, 1, d_model), bf16),
            pltpu.VMEM((AK + 1, U, dh), bf16),
            pltpu.VMEM((AV + 1, U, dh), bf16),
            pltpu.VMEM((n_kv, d_model, hw), bf16),
            pltpu.VMEM((n_kv, d_model, hw), bf16),
            pltpu.VMEM((d_model, ffn), bf16),
            pltpu.VMEM((d_model, ffn), bf16),
            pltpu.VMEM((d_model, ffn), bf16),
            pltpu.VMEM((8, d_model), bf16),
            pltpu.VMEM((n_kv, 8, dh), bf16),
            pltpu.VMEM((8, d_model), jnp.float32),
            pltpu.SemaphoreType.DMA((AK + 1,)),
            pltpu.SemaphoreType.DMA((AV + 1, ns)),
            pltpu.SemaphoreType.DMA((n_kv,)),
            pltpu.SemaphoreType.DMA((n_kv,)),
            pltpu.SemaphoreType.DMA((6,)),
        ],
        compiler_params=pltpu.CompilerParams(vmem_limit_bytes=64 * 1024 * 1024,
                                             disable_bounds_checks=True,
                                             disable_semaphore_checks=True),
    )(A_x, k2, v2, A_wq, wot, B_w_r, B_w_gate, B_w_up, wdt)
```

```python
import functools

import jax
import jax.numpy as jnp
import jax.experimental.pallas as pl
import jax.experimental.pallas.tpu as pltpu


HI = 0
LO = 1

U = 512
KP = (56, 128, 128, 120, 80)
KEV = (0, 1, 3, 4, 5)
VP = (48, 120, 24, 112, 120, 88)
AK = 3
AV = 7
XEV = 0
QK_EV = 0
SM_EV = 1
CB = 256
WD_LAST = 64
NFIN = 3
NEG = -1e30


def _kernel(x_hbm, k_hbm, v_hbm, wq_hbm, wot_hbm, wr_hbm, wg_hbm, wu_hbm, wdt_hbm,
            o_hbm,
            xbuf, wrbuf, obuf, kbuf, vbuf, wqbuf, wobuf, wgbuf, wubuf, wdbuf,
            xn_scr, q_scr, out_scr, hid_scr, rs_scr,
            ksem, vsem, wqsem, wosem, msem,
            *, n_kv, sk, dh, d_model):
    ns = len(VP)
    nkp = len(KP)
    assert len(KEV) == nkp and max(KEV) < ns and sum(KP) == U and sum(VP) == U
    kstarts = [sum(KP[:j]) for j in range(nkp)]
    vstarts = [sum(VP[:j]) for j in range(ns)]
    nb = U // CB
    upb = sk // U
    n_units = n_kv * upb
    nk = AK + 1
    nv = AV + 1
    hw = 2 * dh
    f32 = jnp.float32
    bf16 = jnp.bfloat16
    nt_dims = (((1,), (1,)), ((), ()))

    def k_copy(u, j):
        slot = u % nk
        return pltpu.make_async_copy(
            k_hbm.at[pl.ds(u * U + kstarts[j], KP[j])],
            kbuf.at[slot, pl.ds(kstarts[j], KP[j])], ksem.at[slot])

    def v_copy(u, j):
        slot = u % nv
        return pltpu.make_async_copy(
            v_hbm.at[pl.ds(u * U + vstarts[j], VP[j])],
            vbuf.at[slot, pl.ds(vstarts[j], VP[j])], vsem.at[slot, j])

    def wait_all(buf, sem):
        pltpu.make_async_copy(buf, buf, sem).wait()

    def k_wait(u):
        wait_all(kbuf.at[u % nk], ksem.at[u % nk])

    n_rg = d_model // 8
    n_w16 = d_model // 16
    d_early = d_model - WD_LAST
    n_ffn = 2 * n_rg + d_early // 8
    ffn_per_head = n_ffn // n_kv
    n_extra = 2 * n_w16 + ffn_per_head
    assert ffn_per_head * n_kv == n_ffn and n_extra <= upb - upb // 4 and n_w16 <= upb // 2
    assert d_early % 128 == 0

    def head_piece(src, dst, sem, h, i):
        col = pl.multiple_of(h * hw, hw)
        row = pl.multiple_of(i * 16, 16)
        return pltpu.make_async_copy(src.at[pl.ds(row, 16), pl.ds(col, hw)],
                                     dst.at[h, pl.ds(row, 16)], sem.at[h])

    def ffn_piece(src, dst, sem, i):
        row = pl.multiple_of(i * 8, 8)
        return pltpu.make_async_copy(src.at[pl.ds(row, 8)], dst.at[pl.ds(row, 8)], sem)

    def issue_weight_piece(h, r):
        @pl.when(r < n_extra)
        def _():
            @pl.when(jnp.logical_and(r < n_w16, h < n_kv - 1))
            def _():
                head_piece(wq_hbm, wqbuf, wqsem, h + 1, r).start(priority=HI)

            @pl.when(jnp.logical_and(r >= n_w16, r < 2 * n_w16))
            def _():
                head_piece(wot_hbm, wobuf, wosem, h, r - n_w16).start(priority=HI)

            f = h * ffn_per_head + r - 2 * n_w16

            @pl.when(r >= 2 * n_w16)
            def _():
                @pl.when(f < n_rg)
                def _():
                    ffn_piece(wg_hbm, wgbuf, msem.at[2], f).start(priority=HI)

                @pl.when(jnp.logical_and(f >= n_rg, f < 2 * n_rg))
                def _():
                    ffn_piece(wu_hbm, wubuf, msem.at[3], f - n_rg).start(priority=HI)

                @pl.when(f >= 2 * n_rg)
                def _():
                    ffn_piece(wdt_hbm, wdbuf, msem.at[4], f - 2 * n_rg).start(priority=HI)

    x_copy = pltpu.make_async_copy(x_hbm, xbuf, msem.at[0])
    wr_copy = pltpu.make_async_copy(wr_hbm, wrbuf, msem.at[1])
    wq0_copy = pltpu.make_async_copy(wq_hbm.at[:, pl.ds(0, hw)], wqbuf.at[0], wqsem.at[0])
    out_copy = pltpu.make_async_copy(obuf, o_hbm, msem.at[5])
    wd_last_copy = pltpu.make_async_copy(wdt_hbm.at[pl.ds(d_early, WD_LAST)],
                                         wdbuf.at[pl.ds(d_early, WD_LAST)], msem.at[6])

    x_copy.start(priority=HI)
    wr_copy.start(priority=HI)
    wq0_copy.start(priority=HI)

    def k_init(u, c):
        for j in range(nkp):
            k_copy(u, j).start(priority=HI)
        return c

    def v_init(u, c):
        for j in range(ns):
            v_copy(u, j).start(priority=LO)
        return c

    jax.lax.fori_loop(0, AK + 1, k_init, 0)
    jax.lax.fori_loop(0, AV, v_init, 0)

    x_copy.wait()
    x = xbuf[0].astype(f32)
    mu = jnp.mean(x, axis=1, keepdims=True)
    xc = x - mu
    var = jnp.mean(xc * xc, axis=1, keepdims=True)
    xn = (xc / jnp.sqrt(var + 1e-5)).astype(bf16)
    xn_scr[...] = jnp.broadcast_to(xn, (8, d_model))

    row = jax.lax.broadcasted_iota(jnp.int32, (8, dh), 0)
    top = row < 4

    def make_q(h):
        qf = jnp.dot(xn_scr[...], wqbuf[h], preferred_element_type=f32)
        qh = jnp.where(top, qf[:, :dh], qf[:, dh:]).astype(bf16)
        q_scr[h] = (qh.astype(f32) * (dh ** -0.5)).astype(bf16)

    wq0_copy.wait()
    make_q(0)
    out_scr[...] = jnp.zeros(out_scr.shape, f32)

    def qk(u):
        q = q_scr[u // upb]
        return [jax.lax.dot_general(q, kbuf[u % nk, pl.ds(b * CB, CB), :], nt_dims,
                                    preferred_element_type=f32) for b in range(nb)]

    def softmax(first, s_parts, m, l):
        if first is not None:
            m = jnp.where(first, NEG, m)
            l = jnp.where(first, 0.0, l)
        s = jnp.concatenate(s_parts, axis=1)
        m_new = jnp.maximum(m, jnp.max(s, axis=1, keepdims=True))
        p = jnp.exp(s - m_new)
        alpha = jnp.exp(m - m_new)
        ps = p[:, 0:128]
        for c in range(1, s.shape[1] // 128):
            ps = ps + p[:, c * 128:(c + 1) * 128]
        return p.astype(bf16), alpha, m_new, alpha * l + ps

    def pv(u, p):
        res = None
        for b in range(nb):
            t = jnp.dot(p[:, b * CB:(b + 1) * CB], vbuf[u % nv, pl.ds(b * CB, CB), :],
                        preferred_element_type=f32)
            res = t if res is None else res + t
        return res

    def project(h, o):
        lhs = jnp.concatenate([jnp.where(row == 0, o, 0.0), jnp.where(row == 4, o, 0.0)],
                              axis=1).astype(bf16)
        return jax.lax.dot_general(lhs, wobuf[h], nt_dims, preferred_element_type=f32)

    def ffn():
        wait_all(wgbuf, msem.at[2])
        wait_all(wubuf, msem.at[3])
        wait_all(wdbuf.at[pl.ds(0, d_early)], msem.at[4])
        wr_copy.wait()
        xb = xn_scr[...]
        g = jnp.dot(xb, wgbuf[...], preferred_element_type=f32).astype(bf16).astype(f32)
        up = jnp.dot(xb, wubuf[...], preferred_element_type=f32).astype(bf16).astype(f32)
        g = (g * jax.nn.sigmoid(g)).astype(bf16)
        hid = (g.astype(f32) * up).astype(bf16)
        hid_scr[...] = hid
        y = jax.lax.dot_general(hid, wdbuf[pl.ds(0, d_early), :], nt_dims,
                                preferred_element_type=f32)
        xf = xb.astype(f32)
        wr = wrbuf[...].astype(f32).reshape(1, d_model)
        rs = jax.nn.sigmoid(jnp.sum(xf * wr, axis=1, keepdims=True))
        rs_scr[...] = jnp.broadcast_to(rs, rs_scr.shape)
        rows = jax.lax.broadcasted_iota(jnp.int32, (8, d_model), 0)
        yfull = jnp.concatenate([y * rs, jnp.zeros((8, WD_LAST), f32)], axis=1)
        base = xbuf[0].astype(f32) + xf + xf * 0.0 + yfull
        out_scr[...] += jnp.where(rows == 0, base, 0.0)

    k_wait(0)
    p0, a0, m0, l0 = softmax(None, qk(0), jnp.full((8, 1), NEG, f32), jnp.zeros((8, 128), f32))
    acc0 = jnp.zeros((8, dh), f32)

    def body(u, carry):
        p, alpha, m, l, acc = carry
        h = u // upb
        r = u % upb
        issue_k = u + 1 + AK < n_units
        issue_v = u + AV < n_units
        for j in range(ns):
            v_copy(u, j).wait()
            for jk in range(nkp):
                if KEV[jk] == j:
                    @pl.when(issue_k)
                    def _():
                        k_copy(u + 1 + AK, jk).start(priority=HI)

            @pl.when(issue_v)
            def _():
                v_copy(u + AV, j).start(priority=LO)

            if j == ns - 1:
                @pl.when(u + AV == n_units - 1)
                def _():
                    wd_last_copy.start(priority=LO)
            if j == XEV:
                issue_weight_piece(h, r)
            if j == QK_EV:
                k_wait(u + 1)
                s_parts = qk(u + 1)
            if j == SM_EV:
                nxt = softmax((u + 1) % upb == 0, s_parts, m, l)
        acc = alpha * acc + pv(u, p)

        @pl.when(jnp.logical_and(r == upb // 2, h < n_kv - 1))
        def _():
            wait_all(wqbuf.at[h + 1], wqsem.at[h + 1])
            make_q(h + 1)

        @pl.when(u == n_units - upb // 4)
        def _():
            ffn()

        @pl.when(r == upb - 1)
        def _():
            o = acc / jnp.sum(l, axis=1, keepdims=True)
            wait_all(wobuf.at[h], wosem.at[h])
            out_scr[...] += project(h, o)
        return nxt + (acc,)

    assert 1 <= NFIN <= upb // 4
    carry = jax.lax.fori_loop(0, n_units - NFIN, body, (p0, a0, m0, l0, acc0))

    p, alpha, m, l, acc = carry
    u0 = n_units - NFIN
    if NFIN > 1:
        s_parts = []
        for u in range(u0 + 1, n_units):
            k_wait(u)
            s_parts += qk(u)
        p2, alpha2, _, l = softmax(None, s_parts, m, l)
    rinv = 1.0 / jnp.sum(l, axis=1, keepdims=True)
    wait_all(wobuf.at[n_kv - 1], wosem.at[n_kv - 1])
    acc = alpha * acc
    for j in range(ns):
        v_copy(u0, j).wait()
    acc = acc + pv(u0, p)
    if NFIN > 1:
        acc = alpha2 * acc
    for i, u in enumerate(range(u0 + 1, n_units)):
        for j in range(ns):
            v_copy(u, j).wait()
        acc = acc + pv(u, p2[:, i * U:(i + 1) * U])
    tot = out_scr[...] + project(n_kv - 1, acc * rinv)
    res = jnp.sum(tot, axis=0, keepdims=True)
    wd_last_copy.wait()
    y_last = jax.lax.dot_general(hid_scr[...], wdbuf[pl.ds(d_early, WD_LAST), :], nt_dims,
                                 preferred_element_type=f32) * rs_scr[:, 0:WD_LAST]
    res = res + jnp.concatenate([jnp.zeros((1, d_early), f32), y_last[0:1, :]], axis=1)
    obuf[0] = res.astype(obuf.dtype)
    out_copy.start()
    out_copy.wait()


@jax.jit
def pallas_parallel_sum__gqa_block_cached__moe_arch_mod__decode_kernel(
    A_x: jax.Array,
    A_k_cache: jax.Array,
    A_v_cache: jax.Array,
    A_wq: jax.Array,
    A_wo: jax.Array,
    B_x: jax.Array,
    B_w_r: jax.Array,
    B_w_gate: jax.Array,
    B_w_up: jax.Array,
    B_w_down: jax.Array,
):
    del B_x
    _, n_kv, sk, dh = A_k_cache.shape
    d_model = A_x.shape[-1]
    assert A_wq.shape[1] == 2 * n_kv * dh and A_x.shape == (1, 1, d_model)
    ffn = B_w_gate.shape[1]
    hw = 2 * dh
    ns = len(VP)
    bf16 = jnp.bfloat16

    k2 = A_k_cache.reshape(n_kv * sk, dh)
    v2 = A_v_cache.reshape(n_kv * sk, dh)
    wot = A_wo.T
    wdt = B_w_down.T

    kernel = functools.partial(_kernel, n_kv=n_kv, sk=sk, dh=dh, d_model=d_model)
    return pl.pallas_call(
        kernel,
        out_shape=jax.ShapeDtypeStruct((1, 1, d_model), A_x.dtype),
        in_specs=[pl.BlockSpec(memory_space=pl.ANY)] * 9,
        out_specs=pl.BlockSpec(memory_space=pl.ANY),
        scratch_shapes=[
            pltpu.VMEM((1, 1, d_model), bf16),
            pltpu.VMEM((d_model,), bf16),
            pltpu.VMEM((1, 1, d_model), bf16),
            pltpu.VMEM((AK + 1, U, dh), bf16),
            pltpu.VMEM((AV + 1, U, dh), bf16),
            pltpu.VMEM((n_kv, d_model, hw), bf16),
            pltpu.VMEM((n_kv, d_model, hw), bf16),
            pltpu.VMEM((d_model, ffn), bf16),
            pltpu.VMEM((d_model, ffn), bf16),
            pltpu.VMEM((d_model, ffn), bf16),
            pltpu.VMEM((8, d_model), bf16),
            pltpu.VMEM((n_kv, 8, dh), bf16),
            pltpu.VMEM((8, d_model), jnp.float32),
            pltpu.VMEM((8, ffn), bf16),
            pltpu.VMEM((8, 128), jnp.float32),
            pltpu.SemaphoreType.DMA((AK + 1,)),
            pltpu.SemaphoreType.DMA((AV + 1, ns)),
            pltpu.SemaphoreType.DMA((n_kv,)),
            pltpu.SemaphoreType.DMA((n_kv,)),
            pltpu.SemaphoreType.DMA((7,)),
        ],
        compiler_params=pltpu.CompilerParams(vmem_limit_bytes=64 * 1024 * 1024,
                                             disable_bounds_checks=True,
                                             disable_semaphore_checks=True),
    )(A_x, k2, v2, A_wq, wot, B_w_r, B_w_gate, B_w_up, wdt)
```
